```python
import os as _os
_os.environ.setdefault('JAX_PLATFORMS', 'cpu')
import jax
import jax.numpy as jnp

def _softmax(x, axis=-1):
    return jax.nn.softmax(x, axis=axis)

def _gelu(x):
    return jax.nn.gelu(x, approximate=True)

def _silu(x):
    return jax.nn.silu(x)

def _sigmoid(x):
    return jax.nn.sigmoid(x)

def _layernorm(x, axis=-1, eps=1e-05):
    m = jnp.mean(x, axis=axis, keepdims=True)
    v = jnp.var(x, axis=axis, keepdims=True)
    return (x - m) / jnp.sqrt(v + eps)

def _scatter_add(tgt, idx, src, axis=0):
    return tgt.at[idx].add(src)

def _segment_sum(src, seg, n):
    return jax.ops.segment_sum(src, seg, n)

class _Rng:

    def __init__(self, key):
        self._k = key

    def _next(self):
        self._k, sub = jax.random.split(self._k)
        return sub

    def normal(self, shape):
        return jax.random.normal(self._next(), shape, dtype=jnp.bfloat16)

    def randint(self, lo, hi, shape):
        return jax.random.randint(self._next(), shape, lo, hi, dtype=jnp.int32)

    def uniform(self, shape, lo=0.0, hi=1.0):
        return jax.random.uniform(self._next(), shape, jnp.bfloat16, lo, hi)

    def permutation(self, n):
        return jax.random.permutation(self._next(), n)
kernel_name = 'adaLN_cond__sliding_local_dilated__glu_gated_swiglu__prompt'

def setup_inputs():
    _rng = _Rng(jax.random.key(int.from_bytes(__import__("os").urandom(4), "little")))
    _w = lambda a: (lambda t: t.astype(jnp.bfloat16) if jnp.issubdtype(t.dtype, jnp.floating) else t)(jnp.asarray(a))

    def _A_setup():
        B, S, D = (1, 2048, 576)
        return {'x': _w((lambda *s: _rng.normal(s) * 0.05)(B, S, D)), 'wqkv': _w((lambda *s: _rng.normal(s) * 0.05)(D, 3 * D)), 'wo': _w((lambda *s: _rng.normal(s) * 0.05)(D, D))}
    _A_in = _A_setup()

    def _B_setup():
        B, S, D, F = (1, 2048, 576, 4608)
        return {'x': _w((lambda *s: _rng.normal(s) * 0.05)(B, S, D)), 'w1': _w((lambda *s: _rng.normal(s) * 0.8)(D, F) * (2.0 / D) ** 0.5), 'w3': _w((lambda *s: _rng.normal(s) * 0.8)(D, F) * (2.0 / D) ** 0.5), 'w2': _w((lambda *s: _rng.normal(s) * 0.8)(F, D) * (2.0 / F) ** 0.5)}
    _B_in = _B_setup()
    return {'A_x': _A_in['x'], 'A_wqkv': _A_in['wqkv'], 'A_wo': _A_in['wo'], 'B_x': _B_in['x'], 'B_w1': _B_in['w1'], 'B_w3': _B_in['w3'], 'B_w2': _B_in['w2'], 'c': _w((lambda *s: _rng.normal(s) * 0.05)(1, 576) * 8.0), 'w_mod': _w((lambda *s: _rng.normal(s) * 0.05)(576, 6 * 576) * 576 ** (-0.5) * 8.0)}

def reference(A_x, A_wqkv, A_wo, B_x, B_w1, B_w3, B_w2, c, w_mod):

    def _A_ref(x, wqkv, wo):
        B, S, D = x.shape
        H = 32
        Dh = D // H
        W, dil = (8, 2)
        qkv = (lambda x, *d: x.transpose(*d))((x @ wqkv).reshape(B, S, 3, H, Dh), 2, 0, 3, 1, 4)
        q, k, v = (qkv[0], qkv[1], qkv[2])
        scale = Dh ** (-0.5)
        pos = jnp.arange(S)
        off = jnp.arange(W) * dil
        idx = pos[:, None] - off[None, :]
        mask = idx >= 0
        idx_c = jnp.where(mask, idx, 0).reshape(-1)
        kg = k[:, :, idx_c, :].reshape(B, H, S, W, Dh)
        vg = v[:, :, idx_c, :].reshape(B, H, S, W, Dh)
        logits = jnp.einsum('bhsd,bhswd->bhsw', q, kg) * scale
        logits = jnp.where(mask[None, None, :, :], logits, -1000000000.0)
        attn = _softmax(logits, axis=-1)
        o = jnp.einsum('bhsw,bhswd->bhsd', attn, vg)
        return (lambda x, *d: x.transpose(*d))(o, 0, 2, 1, 3).reshape(B, S, D) @ wo

    def _B_ref(x, w1, w3, w2):
        gate = jnp.einsum('bsd,df->bsf', x, w1)
        up = jnp.einsum('bsd,df->bsf', x, w3)
        h = _silu(gate) * up
        out = jnp.einsum('bsf,fd->bsd', h, w2)
        return out
    x = A_x
    mod = (_silu(c) @ w_mod).reshape(c.shape[0], 6, 1, -1)
    sa, ca, ga, sb, cb, gb = (mod[:, 0].copy(), mod[:, 1].copy(), mod[:, 2].copy(), mod[:, 3].copy(), mod[:, 4].copy(), mod[:, 5].copy())
    h = _layernorm(x, axis=-1) * (1 + ca) + sa
    x = x + ga * _A_ref(h, A_wqkv, A_wo)
    h = _layernorm(x, axis=-1) * (1 + cb) + sb
    x = x + gb * _B_ref(h, B_w1, B_w3, B_w2)
    return x
```

```python
import functools, math
import numpy as np
import jax, jax.numpy as jnp
from jax import lax
from jax.experimental import pallas as pl
from jax.experimental.pallas import tpu as pltpu

S, D, F = 2048, 576, 4608
H, DH, W, DIL = 32, 18, 8, 2
DP = 640
NQ = 14 * 128
NT = (((1,), (1,)), ((), ()))
f32, bf16 = jnp.float32, jnp.bfloat16
LOG2E = math.log2(math.e)
EPS = 1e-5
HALO = 16

def _group_src(t, g):
    if t < 12:
        return (t // 4) * D + (t % 4) * 4 + g
    if t == 12:
        return 16 + g if g < 2 else 2 * D + 14 + g
    return D + 16 + g if g < 2 else -1


def _ln_T(x):
    m = jnp.sum(x, axis=0, keepdims=True) * (1.0 / D)
    xc = x - m
    v = jnp.sum(xc * xc, axis=0, keepdims=True) * (1.0 / D)
    return xc * lax.rsqrt(v + EPS)


def make(TM=256, RC=16, WQ_CH=(4, 4, 3, 3), skip_ffn=False):
    nT = S // TM

    def kern(xt_hbm, wqkv_hbm, wo_hbm, w1_hbm, w3_hbm, w2t_hbm, c_hbm, wmod_hbm, o_ref,
             xt_s, wraw_s, tmp_s, wqt_s, wo_s, wot_s, c_s, wmod_s, w1_s, w3_s, w2t_s,
             mod_s, gcol_s, q_s, kv_s, h_s, o_s, x1_s, h2_s, x1n_s, h2n_s, sems):
        i = pl.program_id(0)

        def x_copy(j):
            return pltpu.make_async_copy(xt_hbm.at[:, pl.ds(j * TM, TM)], xt_s.at[j], sems.at[j])

        bounds = np.cumsum((0,) + WQ_CH)
        def wq_copy(n):
            lo, hi = int(bounds[n]) * 128, min(int(bounds[n + 1]) * 128, 3 * D)
            return pltpu.make_async_copy(wqkv_hbm.at[:, lo:hi], wraw_s.at[:, lo:hi], sems.at[nT + n])
        b = nT + len(WQ_CH)
        c_copy = pltpu.make_async_copy(c_hbm, c_s, sems.at[b])
        wm1_copy = pltpu.make_async_copy(wmod_hbm.at[:, :2 * D], wmod_s.at[:, :2 * D], sems.at[b + 1])
        wm2_copy = pltpu.make_async_copy(wmod_hbm.at[:, 2 * D:], wmod_s.at[:, 2 * D:], sems.at[b + 2])
        wo_copy = pltpu.make_async_copy(wo_hbm, wo_s, sems.at[b + 3])
        w1_copy = pltpu.make_async_copy(w1_hbm, w1_s, sems.at[b + 4])
        w3_copy = pltpu.make_async_copy(w3_hbm, w3_s, sems.at[b + 5])
        w2_copy = pltpu.make_async_copy(w2t_hbm, w2t_s, sems.at[b + 6])

        def norm_rows(xt):
            n = _ln_T(xt)
            n = jnp.concatenate([n, jnp.zeros((DP - D, TM), f32)], axis=0)
            return n.T

        def modulate(n, k):
            return (n * mod_s[2 * k, 0:1, :] + mod_s[2 * k + 1, 0:1, :]).astype(bf16)

        def padrow(r):
            return jnp.concatenate([r, jnp.zeros((8, DP - D), f32)], axis=1)

        def qkv_tile(j, h):
            qkv = lax.dot_general(h, wqt_s[...], NT, preferred_element_type=f32)
            qs = DH ** -0.5 * LOG2E
            tile = lambda t: qkv[:, t * 128:(t + 1) * 128]
            for t, src in enumerate((0, 1, 2, 3, 12)):
                q_s[j, t] = tile(src) * qs
            for t, src in enumerate((4, 5, 6, 7, 13, 8, 9, 10, 11, 12)):
                kv_s[j, t, HALO:, :] = tile(src)
                kv_s[j + 1, t, :HALO, :] = tile(src)[TM - HALO:]

        def attn_tile(j, x1_dst, h2_dst):
            for r in range(TM // RC):
                r0 = r * RC
                q = [q_s[j, t, r0:r0 + RC, :] for t in range(5)]
                ls = []
                for w in range(W):
                    a = HALO + r0 - DIL * w
                    p = q[0] * kv_s[j, 0, a:a + RC, :]
                    for t in range(1, 5):
                        p = p + q[t] * kv_s[j, t, a:a + RC, :]
                    p = p + pltpu.roll(p, 64, 1)
                    p = p + pltpu.roll(p, 32, 1)
                    if r0 < HALO and w > 0:
                        pos = j * TM + r0 + lax.broadcasted_iota(jnp.int32, (RC, 128), 0)
                        p = jnp.where(pos >= DIL * w, p, -1e9 * LOG2E)
                    ls.append(p)
                m = ls[0]
                for w in range(1, W):
                    m = jnp.maximum(m, ls[w])
                es = [jnp.exp2(l - m) for l in ls]
                den = es[0]
                for w in range(1, W):
                    den = den + es[w]
                inv = 1.0 / den
                for t in range(5):
                    acc = None
                    for w in range(W):
                        a = HALO + r0 - DIL * w
                        term = es[w] * kv_s[j, 5 + t, a:a + RC, :]
                        acc = term if acc is None else acc + term
                    o_s[r0:r0 + RC, t * 128:(t + 1) * 128] = (acc * inv).astype(bf16)
            attn_t = lax.dot_general(wot_s[...], o_s[...], NT, preferred_element_type=f32)
            ga = jnp.concatenate([gcol_s[0]] * (TM // 128), axis=1)
            x1 = xt_s[j].astype(f32) + ga * attn_t
            x1_dst[...] = x1
            h2_dst[...] = modulate(norm_rows(x1), 1)

        @pl.when(i == 0)
        def _():
            x_copy(0).start()
            for n in range(len(WQ_CH)):
                wq_copy(n).start()
            c_copy.start()
            wm1_copy.start()
            for j in range(1, nT):
                x_copy(j).start()
            wo_copy.start()
            wm2_copy.start()
            w1_copy.start()
            w3_copy.start()
            w2_copy.start()

            kv_s[0, :, :HALO, :] = jnp.zeros((10, HALO, 128), f32)
            x_copy(0).wait()
            n0 = norm_rows(xt_s[0].astype(f32))
            for n in range(len(WQ_CH)):
                wq_copy(n).wait()
                for s in range(int(bounds[n]), int(bounds[n + 1])):
                    if s < 13:
                        blk = wraw_s[:, s * 128:(s + 1) * 128].astype(f32)
                    else:
                        blk = jnp.concatenate([wraw_s[:, s * 128:].astype(f32), jnp.zeros((D, 64), f32)], axis=1)
                    blk = jnp.concatenate([blk, jnp.zeros((DP - D, 128), f32)], axis=0)
                    bt = blk.T
                    for cc in range(5):
                        tmp_s[cc, s * 128:(s + 1) * 128, :] = bt[:, cc * 128:(cc + 1) * 128]
            for t in range(14):
                for g in range(4):
                    s0 = _group_src(t, g)
                    for cc in range(5):
                        if s0 >= 0:
                            v = tmp_s[cc, pl.ds(s0, H, stride=DH), :]
                        else:
                            v = jnp.zeros((H, 128), f32)
                        wqt_s[t * 128 + g * 32:t * 128 + (g + 1) * 32, cc * 128:(cc + 1) * 128] = v.astype(bf16)
            c_copy.wait()
            c = c_s[...].astype(f32)
            sc = c * jax.nn.sigmoid(c)
            scb = jnp.broadcast_to(sc, (8, D)).astype(bf16)
            wm1_copy.wait()
            mod = jnp.dot(scb, wmod_s[:, :2 * D], preferred_element_type=f32)
            mod_s[0] = padrow(1.0 + mod[:, D:2 * D])
            mod_s[1] = padrow(mod[:, :D])
            h0 = modulate(n0, 0)

            def abody(j, h):
                x_copy(j + 1).wait()
                qkv_tile(j, h)
                return modulate(norm_rows(xt_s[j + 1].astype(f32)), 0)
            h_last = lax.fori_loop(0, nT - 1, abody, h0)

            wm2_copy.wait()
            wo_copy.wait()
            mod = jnp.dot(scb, wmod_s[:, 2 * D:], preferred_element_type=f32)
            mod_s[2] = padrow(0.5 + 0.5 * mod[:, 2 * D:3 * D])
            mod_s[3] = padrow(0.5 * mod[:, D:2 * D])
            for n, (lo, sc_) in enumerate(((0, 1.0), (3 * D, 2.0))):
                g = padrow(mod[:, lo:lo + D] * sc_)
                gb = jnp.broadcast_to(g[0:1], (128, DP))
                gcol_s[n] = gb.T[:D]
            for cc in range(5):
                if cc < 4:
                    tmp_s[cc, :D, :] = wo_s[:, cc * 128:(cc + 1) * 128].astype(f32)
                else:
                    tmp_s[cc, :D, :] = jnp.concatenate([wo_s[:, cc * 128:].astype(f32), jnp.zeros((D, 64), f32)], axis=1)
            for t in range(5):
                rows = []
                for g in range(4):
                    s0 = _group_src(8 + t, g) - 2 * D
                    if s0 >= 0:
                        rows.append(jnp.concatenate([tmp_s[cc, pl.ds(s0, H, stride=DH), :] for cc in range(5)], axis=1))
                    else:
                        rows.append(jnp.zeros((H, DP), f32))
                blk = jnp.concatenate(rows, axis=0)
                wot_s[:, t * 128:(t + 1) * 128] = blk.T[:D].astype(bf16)
            qkv_tile(nT - 1, h_last)
            attn_tile(0, x1n_s, h2n_s)
            w1_copy.wait()
            w3_copy.wait()
            w2_copy.wait()

        x1_s[...] = x1n_s[...]
        h2_s[...] = h2n_s[...]
        if not skip_ffn:
            h2 = h2_s[:, :D]
            g = jnp.dot(h2, w1_s[...], preferred_element_type=f32)
            u = jnp.dot(h2, w3_s[...], preferred_element_type=f32)
            a = (g * u) * (1.0 + jnp.tanh(g))
            y = lax.dot_general(w2t_s[...], a.astype(bf16), NT, preferred_element_type=f32)
            gb = jnp.concatenate([gcol_s[1]] * (TM // 128), axis=1)
            o_ref[...] = (x1_s[...] + gb * y).astype(o_ref.dtype)
            attn_tile(jnp.minimum(i + 1, nT - 1), x1n_s, h2n_s)
        else:
            o_ref[...] = x1_s[...].astype(o_ref.dtype)

    def fn(A_x, A_wqkv, A_wo, B_x, B_w1, B_w3, B_w2, c, w_mod):
        xt = A_x[0].T
        hbm = pl.BlockSpec(memory_space=pltpu.HBM)
        V = pltpu.VMEM
        o = pl.pallas_call(
            kern,
            grid=(nT,),
            in_specs=[hbm] * 8,
            out_specs=pl.BlockSpec((D, TM), lambda i: (0, i)),
            out_shape=jax.ShapeDtypeStruct((D, S), bf16),
            scratch_shapes=[
                V((nT, D, TM), bf16), V((D, 3 * D), bf16), V((5, NQ, 128), f32), V((NQ, DP), bf16),
                V((D, D), bf16), V((D, DP), bf16), V((1, D), bf16), V((D, 6 * D), bf16),
                V((D, F), bf16), V((D, F), bf16), V((D, F), bf16),
                V((4, 8, DP), f32), V((2, D, 128), f32),
                V((nT, 5, TM, 128), f32), V((nT + 1, 10, TM + HALO, 128), f32),
                V((TM, DP), bf16), V((TM, DP), bf16), V((D, TM), f32), V((TM, DP), bf16),
                V((D, TM), f32), V((TM, DP), bf16),
                pltpu.SemaphoreType.DMA((nT + len(WQ_CH) + 7,)),
            ],
            compiler_params=pltpu.CompilerParams(dimension_semantics=("arbitrary",), vmem_limit_bytes=110 * 1024 * 1024),
        )(xt, A_wqkv, A_wo, B_w1, B_w3, B_w2.T, c, w_mod)
        return o.T[None]
    return fn


_impl = make()


@jax.jit
def pallas_adaLN_cond__sliding_local_dilated__glu_gated_swiglu__prompt_kernel(
    A_x: jax.Array,
    A_wqkv: jax.Array,
    A_wo: jax.Array,
    B_x: jax.Array,
    B_w1: jax.Array,
    B_w3: jax.Array,
    B_w2: jax.Array,
    c: jax.Array,
    w_mod: jax.Array,
):
    return _impl(A_x, A_wqkv, A_wo, B_x, B_w1, B_w3, B_w2, c, w_mod)
```

```python
import math
import jax, jax.numpy as jnp
from jax import lax
from jax.experimental import pallas as pl
from jax.experimental.pallas import tpu as pltpu

S, D, F = 2048, 576, 4608
H, DH, W, DIL = 32, 18, 8, 2
DP = 640
NQ = 14 * 128
NT = (((1,), (1,)), ((), ()))
f32, bf16, u32 = jnp.float32, jnp.bfloat16, jnp.uint32
LOG2E = math.log2(math.e)
EPS = 1e-5
HALO = 16
TM = 256
RC = 16
FC = 512
nT = S // TM


def _pair_src(t, g):
    if t < 4:
        return 2 * t + g
    if t == 4:
        return D // 2 + 8 if g == 0 else -1
    if t < 9:
        return D // 2 + 2 * (t - 5) + g
    if t < 13:
        return D + 2 * (t - 9) + g
    return 8 if g == 0 else D + 8


Q_TILES = (0, 1, 2, 3, 13)
KV_TILES = (5, 6, 7, 8, 4, 9, 10, 11, 12, 13)
KCH = (((0, 1), ((0, 1), (4, 6))), ((1, 2), ((1, 2), (6, 7))), ((2, 3), ((2, 3), (7, 8))), ((3, 5), ((3, 4), (8, 9))))


def _tree_sum(parts):
    while len(parts) > 1:
        parts = [parts[k] + parts[k + 1] if k + 1 < len(parts) else parts[k] for k in range(0, len(parts), 2)]
    return parts[0]


def make(QS=((0, 4), (4, 8), (8, 11), (11, 14)), lag=(1, 1, 1), gstep=24, ks=4, lt=1, stop=99):

    def kern(xt_hbm, wqkv_hbm, wo_hbm, w1_hbm, w3_hbm, w2t_hbm, c_hbm, wmod_hbm, o_hbm,
             xt_s, wraw_s, tmp_s, wqt_s, wo_s, wot_s, c_s, wmod_s, w1_s, w3_s, w2t_s,
             mod_s, gcol_s, scol_s, n_s, part_s, q_s, kv_s, ha_s, hb_s, o_s, x1_s, x1n_s, h2n_s,
             zero_s, act_s, out_s, sems):
        cp = pltpu.make_async_copy
        nfin = nT - 2 - (3 if lt == 1 else 4)
        nloop = (nT - 2 - nfin) // lt

        def x_copy(j, sem):
            return cp(xt_hbm.at[:, pl.ds(j * TM, TM)], xt_s.at[j], sems.at[sem])

        g_first = [x_copy(0, 0), x_copy(1, 0), cp(c_hbm, c_s, sems.at[0])]
        g_k = []
        for n, ((k0, k1), mts) in enumerate(KCH):
            g = [cp(wmod_hbm.at[:, a * 128:b * 128], wmod_s.at[:, a * 128:b * 128], sems.at[1 + n]) for a, b in mts]
            g.append(cp(wqkv_hbm.at[k0 * 128:min(k1 * 128, D), :], wraw_s.at[k0 * 128:min(k1 * 128, D), :], sems.at[1 + n]))
            g_k.append(g)
        g_k[3].append(x_copy(2, 4))

        def g_loop(jj):
            return [x_copy(3 + jj * lt + n, 5 + jj) for n in range(lt)]
        b = 5 + nloop
        g_fin = [x_copy(j, b) for j in range(3 + nloop * lt, nT)]
        g_fin += [cp(wo_hbm, wo_s, sems.at[b]), cp(wmod_hbm.at[:, 2 * D:], wmod_s.at[:, 2 * D:], sems.at[b])]
        g_gu = [cp(w1_hbm, w1_s, sems.at[b + 1]), cp(w3_hbm, w3_s, sems.at[b + 1])]
        g_dn = [cp(w2t_hbm, w2t_s, sems.at[b + 2])]
        osem = sems.at[b + 3]

        def start(g):
            for c in g:
                c.start()

        def wait(g):
            for c in g:
                c.wait()

        def ld16(ref, r0, r1, c0=0, c1=None):
            return pltpu.bitcast(ref[r0 // 2:r1 // 2, c0:c1], bf16)

        def st16(ref, r0, r1, sl, v):
            ref[r0 // 2:r1 // 2, sl] = pltpu.bitcast(v, u32)

        def gated(v, gate):
            if gate is None:
                return v
            bits = pltpu.bitcast(v, u32) if v.dtype != u32 else v
            z = gate if bits.shape[0] == 8 else jnp.concatenate([gate] * (bits.shape[0] // 8), axis=0)
            return pltpu.bitcast(bits | z, v.dtype) if v.dtype != u32 else bits | z

        def mkgate(outs):
            z = None
            for ob in outs:
                bb = ob if ob.dtype == u32 else pltpu.bitcast(ob, u32)
                z = bb if z is None else z | bb
            return z & zero_s[...]

        def tie(h, z):
            if z is None:
                return h
            top = gated(h[:16, :128], z)
            if h.shape[1] > 128:
                top = jnp.concatenate([top, h[:16, 128:]], axis=1)
            return jnp.concatenate([top, h[16:]], axis=0)

        def gates(res, t):
            return lambda r: mkgate([res[r:r + 8, t * 128:(t + 1) * 128]])

        def run_slots(dots, plan, lag):
            pend = []
            for k, dot in enumerate(dots):
                z = pend.pop(0) if len(pend) > lag else None
                res = dot(lambda h: tie(h, z))
                new = []
                for task, t in (plan[k] if k < len(plan) else []):
                    new += task(gates(res, t))
                pend.append(mkgate(new) if new else None)

        def rowsum(a):
            return jnp.sum(_tree_sum([a[k:k + 8] for k in range(0, a.shape[0], 8)]), axis=0, keepdims=True)

        def ln_stats(ld, gate):
            piv = ld(0, 8)[0:1]
            piv8 = jnp.broadcast_to(piv, (8, 128))
            a1 = a2 = None
            for n, r in enumerate(range(0, D, 64)):
                p = piv if gate is None else gated(piv8, gate(n * gstep))[0:1]
                v = ld(r, 64) - p
                v1 = v[:32] + v[32:]
                v = v * v
                v2 = v[:32] + v[32:]
                a1 = v1 if a1 is None else a1 + v1
                a2 = v2 if a2 is None else a2 + v2
            s1, s2 = rowsum(a1) * (1.0 / D), rowsum(a2) * (1.0 / D)
            var = jnp.maximum(s2 - s1 * s1, 0.0)
            return piv + s1, lax.rsqrt(var + EPS)

        def ln_norm(ld, m, rstd, t):
            n = min(128, D - t * 128)
            blk = (ld(t * 128, n) - m) * rstd
            if n < 128:
                blk = jnp.concatenate([blk, jnp.zeros((128 - n, 128), f32)], axis=0)
            return blk.T

        def modulate(v, k, sl):
            return (v * mod_s[2 * k, 0:1, sl] + mod_s[2 * k + 1, 0:1, sl]).astype(bf16)

        def ln_apply(ld, m, rstd, k, dst, c):
            outs = []
            for t in range(5):
                sl = slice(t * 128, (t + 1) * 128)
                hb = modulate(ln_norm(ld, m, rstd, t), k, sl)
                st16(dst, c * 128, (c + 1) * 128, sl, hb)
                outs.append(hb[112:])
            return outs

        ALLC = tuple(range(TM // 128))
        ln2_stats = {}

        def xld(j, c):
            return lambda r, n: xt_s[j, r:r + n, c * 128:(c + 1) * 128].astype(f32)

        def ln1(j, dst, c, gate):
            ld = xld(j, c)
            return ln_apply(ld, *ln_stats(ld, gate), 0, dst, c)

        def ln2(c, gate):
            m, rstd = ln2_stats[c]
            m = gated(jnp.broadcast_to(m, (8, 128)), gate(0))[0:1]
            return ln_apply(lambda r, n: x1n_s[r:r + n, c * 128:(c + 1) * 128], m, rstd, 1, h2n_s, c)

        def padrow(r):
            return jnp.concatenate([r, jnp.zeros((r.shape[0], DP - D), f32)], axis=1)

        def colbcast(row):
            return jnp.broadcast_to(row, (128, DP)).T[:D]

        def matvec(t):
            acc = None
            for r in range(0, D, 32):
                v = wmod_s[r:r + 32, t * 128:(t + 1) * 128].astype(f32) * scol_s[r:r + 32, :]
                acc = v if acc is None else acc + v
            return rowsum(acc)

        def qkv_store(j, qkv, t0, t1):
            qs = DH ** -0.5 * LOG2E
            for t in range(t0, t1):
                v = qkv[:, (t - t0) * 128:(t - t0 + 1) * 128]
                if t in Q_TILES:
                    q_s[j, Q_TILES.index(t)] = v * qs
                if t in KV_TILES:
                    kv_s[j, KV_TILES.index(t), HALO:, :] = v
                    kv_s[j + 1, KV_TILES.index(t), :HALO, :] = v[TM - HALO:]

        def qkv_dots(j, src, parts, k0=0, k1=5):
            st = {}

            def mk(t0, t1):
                def dot(tief):
                    if 'h' not in st:
                        st['h'] = ld16(src, 0, TM, k0 * 128, k1 * 128)
                    st['h'] = tief(st['h'])
                    wq = ld16(wqt_s, t0 * 128, t1 * 128, k0 * 128, k1 * 128)
                    res = lax.dot_general(st['h'], wq, NT, preferred_element_type=f32)
                    acc = res if k0 == 0 else res + part_s[j, :, t0 * 128:t1 * 128]
                    if k1 < 5:
                        part_s[j, :, t0 * 128:t1 * 128] = acc
                    else:
                        qkv_store(j, acc, t0, t1)
                    return res
                return dot
            return [mk(*p) for p in parts]

        def attn_chunk(j, r, gate):
            r0 = r * RC
            q = [gated(q_s[j, t, r0:r0 + RC, :], gate) for t in range(5)]
            even = (lax.broadcasted_iota(jnp.int32, (RC, 128), 1) & 1) == 0
            ls = []
            for w in range(W):
                a = HALO + r0 - DIL * w
                p = q[0] * kv_s[j, 0, a:a + RC, :]
                for t in range(1, 5):
                    p = p + q[t] * kv_s[j, t, a:a + RC, :]
                p = p + pltpu.roll(p, 64, 1)
                p = p + jnp.where(even, pltpu.roll(p, 127, 1), pltpu.roll(p, 1, 1))
                if r0 < HALO and w > 0:
                    pos = j * TM + r0 + lax.broadcasted_iota(jnp.int32, (RC, 128), 0)
                    p = jnp.where(pos >= DIL * w, p, -1e9 * LOG2E)
                ls.append(p)
            m = ls[0]
            for w in range(1, W):
                m = jnp.maximum(m, ls[w])
            es = [jnp.exp2(l - m) for l in ls]
            inv = 1.0 / _tree_sum(es)
            outs = []
            for t in range(5):
                acc = None
                for w in range(W):
                    a = HALO + r0 - DIL * w
                    term = es[w] * kv_s[j, 5 + t, a:a + RC, :]
                    acc = term if acc is None else acc + term
                ob = (acc * inv).astype(bf16)
                st16(o_s, r0, r0 + RC, slice(t * 128, (t + 1) * 128), ob)
                outs.append(ob[:16])
            return outs

        def wo_dot(j):
            def dot(tief):
                attn_t = lax.dot_general(tief(ld16(wot_s, 0, D)), ld16(o_s, 0, TM), NT, preferred_element_type=f32)
                ga = jnp.concatenate([gcol_s[0]] * len(ALLC), axis=1)
                x1 = xt_s[j].astype(f32) + ga * attn_t
                x1n_s[...] = x1
                for c in ALLC:
                    ln2_stats[c] = ln_stats(lambda r, m: x1[r:r + m, c * 128:(c + 1) * 128], None)
                return attn_t
            return dot

        def wq_prep(k0, k1):
            r0, r1 = k0 * 128, min(k1 * 128, D)
            for s in range(14):
                if s < 13:
                    blk = wraw_s[r0:r1, s * 128:(s + 1) * 128]
                else:
                    blk = jnp.concatenate([wraw_s[r0:r1, s * 128:], jnp.zeros((r1 - r0, 64), bf16)], axis=1)
                if r1 < k1 * 128:
                    blk = jnp.concatenate([blk, jnp.zeros((k1 * 128 - r1, 128), bf16)], axis=0)
                bt = pltpu.bitcast(blk.T, u32)
                for cc in range(k0, k1):
                    tmp_s[cc, s * 64:(s + 1) * 64, :] = bt[:, (cc - k0) * 128:(cc - k0 + 1) * 128]
            for t in range(14):
                for g in range(2):
                    s0 = _pair_src(t, g)
                    for cc in range(k0, k1):
                        if s0 >= 0:
                            v = tmp_s[cc, pl.ds(s0, H, stride=DH // 2), :]
                        else:
                            v = jnp.zeros((H, 128), u32)
                        wqt_s[t * 64 + g * 32:t * 64 + (g + 1) * 32, cc * 128:(cc + 1) * 128] = v

        def wo_cvt(gate):
            outs = []
            for cc in range(5):
                if cc < 4:
                    v = wo_s[:, cc * 128:(cc + 1) * 128]
                else:
                    v = jnp.concatenate([wo_s[:, cc * 128:], jnp.zeros((D, 64), bf16)], axis=1)
                v = gated(pltpu.bitcast(v, u32), gate(cc * 48))
                tmp_s[cc, :D // 2, :] = v
                outs.append(v[D // 2 - 8:])
            return outs

        def wo_perm(t, gate):
            rows = []
            for g in range(2):
                s0 = _pair_src(9 + t, g) - D
                if s0 >= 0:
                    rows.append(jnp.concatenate(
                        [gated(tmp_s[cc, pl.ds(s0, H, stride=DH // 2), :], gate) for cc in range(5)], axis=1))
                else:
                    rows.append(jnp.zeros((H, DP), u32))
            blk = pltpu.bitcast(jnp.concatenate(rows, axis=0), bf16).T[:D]
            st16(wot_s, 0, D, slice(t * 128, (t + 1) * 128), blk)
            return [blk[k:k + 16] for k in (112, 240, 368, 496, 560)]

        A = lambda j, r: (lambda gt: attn_chunk(j, r, gt(0)))
        L1 = lambda j, dst, c: (lambda gt: ln1(j, dst, c, gt))
        L2 = lambda c: (lambda gt: ln2(c, gt))
        P = lambda t: (lambda gt: wo_perm(t, gt(0)))
        ident = lambda h: h

        start(g_first)
        for g in g_k:
            start(g)
        if stop > 5:
            for jj in range(nloop):
                start(g_loop(jj))
        if stop > 10:
            start(g_fin)
        if stop > 20:
            start(g_gu)
            start(g_dn)

        kv_s[0, :, :HALO, :] = jnp.zeros((10, HALO, 128), f32)
        zero_s[...] = jnp.zeros((8, 128), u32)
        wait(g_first)
        c = c_s[...].astype(f32)
        sc = (c * jax.nn.sigmoid(c)).astype(bf16)
        scol_s[...] = colbcast(padrow(sc.astype(f32)))
        for j in range(2):
            for cc in ALLC:
                ld = xld(j, cc)
                m, rstd = ln_stats(ld, None)
                for t in range(5):
                    n_s[j, cc * 128:(cc + 1) * 128, t * 128:(t + 1) * 128] = ln_norm(ld, m, rstd, t)

        mt = {}

        def kprep(n):
            (k0, k1), mts = KCH[n]
            for a, bb in mts:
                for t in range(a, bb):
                    mt[t] = matvec(t)
            for k in range(k0, k1):
                sl = slice(k * 128, (k + 1) * 128)
                if k < 4:
                    shift = mt[k]
                    scale = 1.0 + jnp.concatenate([mt[4 + k][:, 64:], mt[5 + k][:, :64]], axis=1)
                else:
                    z = jnp.zeros((1, 64), f32)
                    shift = jnp.concatenate([mt[4][:, :64], z], axis=1)
                    scale = jnp.concatenate([1.0 + mt[8][:, 64:], z], axis=1)
                mod_s[0, :, sl] = jnp.broadcast_to(scale, (8, 128))
                mod_s[1, :, sl] = jnp.broadcast_to(shift, (8, 128))
                for j, dst in ((0, ha_s), (1, hb_s)):
                    st16(dst, 0, TM, sl, (n_s[j, :, sl] * scale + shift).astype(bf16))
            wq_prep(k0, k1)

        ALLT = ((0, 14),)
        for n in range(4):
            wait(g_k[n])
            if n > 0:
                qkv_dots(1, hb_s, ALLT, *KCH[n - 1][0])[0](ident)
            kprep(n)
            if n < 3:
                qkv_dots(0, ha_s, ALLT, *KCH[n][0])[0](ident)
        dots = qkv_dots(0, ha_s, ALLT, 3, 5) + qkv_dots(1, hb_s, ((0, 8), (8, 14)), 3, 5)
        run_slots(dots, [[(L1(2, ha_s, 0), 4), (L1(2, ha_s, 1), 9)]], 1)
        if stop == 5:
            return

        def abody(jj, _):
            wait(g_loop(jj))
            j = 2 + lt * jj
            if lt == 1:
                dots = qkv_dots(j, ha_s, QS)
                plan = [[(L1(j + 1, ha_s, 0), 0)], [(L1(j + 1, ha_s, 1), 0)]]
            else:
                dots = qkv_dots(j, ha_s, QS) + qkv_dots(j + 1, hb_s, QS)
                plan = [[(L1(j + 1, hb_s, 0), 0)], [(L1(j + 1, hb_s, 1), 0)], [], [],
                        [(L1(j + 2, ha_s, 0), 0)], [(L1(j + 2, ha_s, 1), 0)], [], []]
            run_slots(dots, plan, lag[0])
            return 0
        lax.fori_loop(0, nloop, abody, 0)
        if stop == 10:
            return

        wait(g_fin)
        scb = jnp.broadcast_to(sc, (8, D))
        mod = jnp.dot(scb, wmod_s[:, 2 * D:], preferred_element_type=f32)
        mod_s[2] = padrow(0.5 + 0.5 * mod[:, 2 * D:3 * D])
        mod_s[3] = padrow(0.5 * mod[:, D:2 * D])
        gcol_s[0] = colbcast(padrow(mod[0:1, :D]))
        gcol_s[1] = colbcast(padrow(2.0 * mod[0:1, 3 * D:]))
        a = lambda r: A(0, r)
        if nfin == 3:
            d7 = qkv_dots(7, ha_s, QS)
            dots = qkv_dots(5, ha_s, QS) + qkv_dots(6, hb_s, QS) + d7[:1] + [wo_dot(0)] + d7[1:]
            plan = [[(L1(6, hb_s, 0), 0), (a(0), 2), (wo_cvt, 3)], [(L1(6, hb_s, 1), 0), (a(1), 2), (a(2), 3)],
                    [(a(3), 0), (P(0), 1), (a(4), 2)], [(a(5), 0), (P(1), 1), (a(6), 2)],
                    [(L1(7, ha_s, 0), 0), (a(7), 1), (P(2), 2), (a(8), 3)],
                    [(L1(7, ha_s, 1), 0), (a(9), 1), (P(3), 2), (a(10), 3)],
                    [(a(11), 0), (P(4), 1), (a(12), 2)], [(a(13), 0), (a(14), 1), (a(15), 2)],
                    [], [], [(L2(0), 0), (L2(1), 2)], [], []]
        else:
            d7 = qkv_dots(7, hb_s, QS)
            dots = qkv_dots(6, ha_s, QS) + d7[:2] + [wo_dot(0)] + d7[2:]
            plan = [[(L1(7, hb_s, 0), 0), (a(0), 1), (wo_cvt, 1), (a(1), 2), (a(2), 3)],
                    [(L1(7, hb_s, 1), 0), (a(3), 1), (P(0), 1), (a(4), 2), (a(5), 3), (P(1), 3)],
                    [(a(6), 0), (a(7), 1), (P(2), 1), (a(8), 2)], [(a(9), 0), (P(3), 0), (a(10), 1), (a(11), 2), (P(4), 2)],
                    [(a(12), 0), (a(13), 1), (a(14), 2), (a(15), 3)], [], [], [(L2(0), 0), (L2(1), 1)], []]
        run_slots(dots, plan, lag[1])
        if stop == 20:
            return
        wait(g_gu)

        def out_copy(i, c0, n):
            return cp(out_s.at[i, :, pl.ds(c0, n)], o_hbm.at[:, pl.ds(i * TM + c0, n)], osem)

        def bbody(i, _):
            jn = jnp.minimum(i + 1, nT - 1)
            x1_s[...] = x1n_s[...]
            st = {'h': ld16(h2n_s, 0, TM, 0, D)}

            def gdot(sl):
                def dot(tief):
                    st['h'] = tief(st['h'])
                    st['g'] = jnp.dot(st['h'], w1_s[:, sl], preferred_element_type=f32)
                    return st['g']
                return dot

            def udot(sl):
                def dot(tief):
                    st['h'] = tief(st['h'])
                    u = jnp.dot(st['h'], w3_s[:, sl], preferred_element_type=f32)
                    g = st['g']
                    st16(act_s, 0, TM, sl, ((g * u) * (1.0 + jnp.tanh(g))).astype(bf16))
                    return u
                return dot
            dots = []
            for cidx in range(F // FC):
                sl = slice(cidx * FC, (cidx + 1) * FC)
                dots += [gdot(sl), udot(sl)]
            run_slots(dots, [[(A(jn, r), 0)] for r in range(TM // RC)], lag[2])

            @pl.when(i == 0)
            def _():
                wait(g_dn)

            @pl.when(i < nT - 1)
            def _():
                wo_dot(jn)(ident)
                w = w2t_s[...]
                KS = ks * 128
                y0 = lax.dot_general(w[:, :KS], ld16(act_s, 0, TM, 0, KS), NT, preferred_element_type=f32)
                outs = ln2(0, gates(y0, 0)) + ln2(1, gates(y0, 1))
                y1 = lax.dot_general(w[:, KS:2 * KS], ld16(act_s, 0, TM, KS, 2 * KS), NT, preferred_element_type=f32)
                y2 = lax.dot_general(tie(w[:, 2 * KS:], mkgate(outs)), ld16(act_s, 0, TM, 2 * KS, F), NT,
                                     preferred_element_type=f32)
                gb = jnp.concatenate([gcol_s[1]] * len(ALLC), axis=1)
                out_s[i] = (x1_s[...] + gb * (y0 + y1 + y2)).astype(bf16)
                out_copy(i, 0, TM).start()
            return 0
        lax.fori_loop(0, nT, bbody, 0)

        def qbody(c, _):
            off = pl.multiple_of(c * 128, 128)
            a = pltpu.bitcast(act_s[pl.ds(pl.multiple_of(c * 64, 64), 64), :], bf16)
            y = lax.dot_general(w2t_s[...], a, NT, preferred_element_type=f32)
            out_s[nT - 1, :, pl.ds(off, 128)] = (x1_s[:, pl.ds(off, 128)] + gcol_s[1] * y).astype(bf16)
            out_copy(nT - 1, off, 128).start()
            return 0
        lax.fori_loop(0, TM // 128, qbody, 0)
        cp(out_s, out_s, osem).wait()

    def fn(A_x, A_wqkv, A_wo, B_x, B_w1, B_w3, B_w2, c, w_mod):
        xt = A_x[0].T
        hbm = pl.BlockSpec(memory_space=pltpu.HBM)
        V = pltpu.VMEM
        o = pl.pallas_call(
            kern,
            in_specs=[hbm] * 8,
            out_specs=hbm,
            out_shape=jax.ShapeDtypeStruct((D, S), bf16),
            scratch_shapes=[
                V((nT, D, TM), bf16), V((D, 3 * D), bf16), V((5, NQ // 2, 128), u32), V((NQ // 2, DP), u32),
                V((D, D), bf16), V((D // 2, DP), u32), V((1, D), bf16), V((D, 6 * D), bf16),
                V((D, F), bf16), V((D, F), bf16), V((D, F), bf16),
                V((4, 8, DP), f32), V((2, D, 128), f32), V((D, 128), f32),
                V((2, TM, DP), f32), V((2, TM, NQ), f32),
                V((nT, 5, TM, 128), f32), V((nT + 1, 10, TM + HALO, 128), f32),
                V((TM // 2, DP), u32), V((TM // 2, DP), u32), V((TM // 2, DP), u32), V((D, TM), f32),
                V((D, TM), f32), V((TM // 2, DP), u32), V((8, 128), u32), V((TM // 2, F), u32),
                V((nT, D, TM), bf16),
                pltpu.SemaphoreType.DMA((12,)),
            ],
            compiler_params=pltpu.CompilerParams(vmem_limit_bytes=110 * 1024 * 1024),
        )(xt, A_wqkv, A_wo, B_w1, B_w3, B_w2.T, c, w_mod)
        return o.T[None]
    return fn


_impl = make()


@jax.jit
def pallas_adaLN_cond__sliding_local_dilated__glu_gated_swiglu__prompt_kernel(
    A_x: jax.Array,
    A_wqkv: jax.Array,
    A_wo: jax.Array,
    B_x: jax.Array,
    B_w1: jax.Array,
    B_w3: jax.Array,
    B_w2: jax.Array,
    c: jax.Array,
    w_mod: jax.Array,
):
    return _impl(A_x, A_wqkv, A_wo, B_x, B_w1, B_w3, B_w2, c, w_mod)
```

```python
import math

import jax
import jax.numpy as jnp
from jax import lax
from jax.experimental import pallas as pl
from jax.experimental.pallas import tpu as pltpu

S, D, F = 2048, 576, 4608
H, DH, W, DIL = 32, 18, 8, 2
DP = 640
NT = (((1,), (1,)), ((), ()))
f32, bf16, u32 = jnp.float32, jnp.bfloat16, jnp.uint32
LOG2E = math.log2(math.e)
EPS = 1e-5
HALO = 16
TM = 256
RC = 16
FC = 512
LC = 256
NB = S // TM
NLOOP = 3
MW = 4 * D // NLOOP


def _pair_src(t, g):
    if t < 12:
        return (t // 4) * (D // 2) + 2 * (t % 4) + g
    if t == 12:
        return 8 if g == 0 else D + 8
    return D // 2 + 8 if g == 0 else -1


Q_TILES = (0, 1, 2, 3, 12)
K_TILES = (4, 5, 6, 7, 13)
V_TILES = (8, 9, 10, 11, 12)
KCH = ((4, (4, 8)), (0, (0, 5)), (1, (1, 6)), (2, (2, 7)), (3, (3,)))
NK = len(KCH)


def _tree_sum(parts):
    while len(parts) > 1:
        parts = [parts[k] + parts[k + 1] if k + 1 < len(parts) else parts[k] for k in range(0, len(parts), 2)]
    return parts[0]


def make(QS=((0, 4), (4, 8), (8, 11), (11, 13)), kt_at=(8, 0, 11, 0), lag=(1, 2, 1), gstep=24, ks=4, pk=8,
         l1g=(0, 4), sh=4, qsp=(0, 256, 448, 576), xpos=(0, 2), wpos=2, lplan='A,.,m,m|B,.,m,m|m,m',
         fplan='V,A,a,a|p,B,a,.|a,M,a|p,a|a,C,.,.|D,a,p,a|a,a,a|p,p|a,a,a,a|.|.|X,.,Y'):

    def kern(xt_hbm, wqkv_hbm, wo_hbm, w1_hbm, w3_hbm, w2t_hbm, c_hbm, wmod_hbm, o_hbm,
             xt_s, wraw_s, tmp_s, wqt_s, wo_s, wot_s, c_s, wmod_s, wm2_s, mraw_s, w1_s, w3_s, w2t_s,
             mod_s, gcol_s, scol_s, part_s, stg_s, kv_s, ha_s, hb_s, hc_s, o_s, x1_s, x1n_s, h2n_s,
             zero_s, act_s, out_s, sems):
        cp = pltpu.make_async_copy

        def x_copy(j, sem):
            return cp(xt_hbm.at[:, pl.ds(j * TM, TM)], xt_s.at[j], sems.at[sem])

        def wq_copy(k, sem):
            rows = slice(k * 128, min((k + 1) * 128, D))
            return cp(wqkv_hbm.at[rows, :], wraw_s.at[rows, :], sems.at[sem])

        g_first = [x_copy(0, 0), cp(c_hbm, c_s, sems.at[0])]
        g_second = [x_copy(1, 1), wq_copy(KCH[0][0], 1)]
        g_k = []
        for n, (k, mts) in enumerate(KCH):
            g = [cp(wmod_hbm.at[:, t * 128:(t + 1) * 128], wmod_s.at[:, t * 128:(t + 1) * 128], sems.at[2 + n])
                 for t in mts]
            if n > 0:
                g.append(wq_copy(k, 2 + n))
            g_k.append(g)
        g_k[NK - 1].append(x_copy(2, NK + 1))

        def g_loop(jj):
            cols = pl.ds(pl.multiple_of(2 * D + jj * MW, 128), MW)
            return [x_copy(3 + jj, NK + 2 + jj), cp(wmod_hbm.at[:, cols], wm2_s.at[jj], sems.at[NK + 2 + jj])]

        g_fin = [x_copy(j, 0) for j in range(3 + NLOOP, NB)] + [cp(wo_hbm, wo_s, sems.at[0])]
        g_gu = [cp(w1_hbm, w1_s, sems.at[1]), cp(w3_hbm, w3_s, sems.at[1])]
        g_dn = [cp(w2t_hbm, w2t_s, sems.at[2])]
        osem = sems.at[3]

        def start(g):
            for c in g:
                c.start()

        def wait(g):
            for c in g:
                c.wait()

        def ld16(ref, r0, r1, c0=0, c1=None):
            return pltpu.bitcast(ref[r0 // 2:r1 // 2, c0:c1], bf16)

        def st16(ref, r0, r1, sl, v):
            bits = pltpu.bitcast(v, u32)
            ref[r0 // 2:r1 // 2, sl] = bits
            return bits

        def gated(v, gate):
            if gate is None:
                return v
            bits = pltpu.bitcast(v, u32) if v.dtype != u32 else v
            z = gate if bits.shape[0] == 8 else jnp.concatenate([gate] * (bits.shape[0] // 8), axis=0)
            return pltpu.bitcast(bits | z, v.dtype) if v.dtype != u32 else bits | z

        def mkgate(outs):
            z = None
            for ob in outs:
                bb = ob if ob.dtype == u32 else pltpu.bitcast(ob, u32)
                z = bb if z is None else z | bb
            return z & zero_s[...]

        def tie(h, z):
            if z is None:
                return h
            top = gated(h[:16, :128], z)
            if h.shape[1] > 128:
                top = jnp.concatenate([top, h[:16, 128:]], axis=1)
            return jnp.concatenate([top, h[16:]], axis=0)

        def gates(res, t):
            return lambda r: mkgate([res[r:r + 8, t * 128:(t + 1) * 128]])

        def run_slots(dots, plan, lag):
            pend = []
            for k, dot in enumerate(dots):
                z = pend.pop(0) if len(pend) > lag else None
                res = dot(lambda h: tie(h, z))
                new = []
                for task, t in (plan[k] if k < len(plan) else []):
                    new += task(gates(res, t))
                pend.append(mkgate(new) if new else None)

        def parse_plan(text, tasks):
            plan = []
            for slot in text.split('|'):
                row = []
                for t, names in enumerate(slot.split(',')):
                    for ch in names.strip('.'):
                        row.append((tasks[ch].pop(0), t))
                plan.append(row)
            assert not any(tasks.values())
            return plan

        def rowsum(a):
            return jnp.sum(_tree_sum([a[k:k + 8] for k in range(0, a.shape[0], 8)]), axis=0, keepdims=True)

        def ln_stats(ld, gate):
            piv = ld(0, 8)[0:1]
            piv8 = jnp.broadcast_to(piv, (8, 128))
            a1 = a2 = None
            for n, r in enumerate(range(0, D, 64)):
                p = piv if gate is None else gated(piv8, gate(n * gstep))[0:1]
                v = ld(r, 64) - p
                v1 = v[:32] + v[32:]
                v = v * v
                v2 = v[:32] + v[32:]
                a1 = v1 if a1 is None else a1 + v1
                a2 = v2 if a2 is None else a2 + v2
            s1, s2 = rowsum(a1) * (1.0 / D), rowsum(a2) * (1.0 / D)
            var = jnp.maximum(s2 - s1 * s1, 0.0)
            return piv + s1, lax.rsqrt(var + EPS)

        def ln_norm(ld, m, rstd, t):
            n = min(128, D - t * 128)
            blk = (ld(t * 128, n) - m) * rstd
            if n < 128:
                blk = jnp.concatenate([blk, jnp.zeros((128 - n, 128), f32)], axis=0)
            return blk.T

        def modulate(v, k, sl):
            return (v * mod_s[2 * k, 0:1, sl] + mod_s[2 * k + 1, 0:1, sl]).astype(bf16)

        def ln_apply(ld, m, rstd, k, dst, c):
            outs = []
            for t in range(5):
                sl = slice(t * 128, (t + 1) * 128)
                hb = modulate(ln_norm(ld, m, rstd, t), k, sl)
                outs.append(st16(dst, c * 128, (c + 1) * 128, sl, hb)[56:])
            return outs

        ALLC = tuple(range(TM // 128))
        ln2_stats = {}

        def xld(j, c):
            return lambda r, n: xt_s[j, r:r + n, c * 128:(c + 1) * 128].astype(f32)

        def ln1(j, dst, c, gate):
            ld = xld(j, c)
            return ln_apply(ld, *ln_stats(ld, gate), 0, dst, c)

        def ln2(c, gate):
            m, rstd = ln2_stats[c]
            m = gated(jnp.broadcast_to(m, (8, 128)), gate(0))[0:1]
            return ln_apply(lambda r, n: x1n_s[r:r + n, c * 128:(c + 1) * 128], m, rstd, 1, h2n_s, c)

        def padrow(r):
            return jnp.concatenate([r, jnp.zeros((r.shape[0], DP - D), f32)], axis=1)

        def colbcast(row):
            return jnp.broadcast_to(row, (128, DP)).T[:D]

        def matvec(ld, gate):
            acc = None
            for n, r in enumerate(range(0, D, 64)):
                sv = scol_s[r:r + 64, :]
                if gate is not None:
                    sv = gated(sv, gate(n * gstep))
                v = ld(r, 64).astype(f32) * sv
                v = v[:32] + v[32:]
                acc = v if acc is None else acc + v
            return rowsum(acc)

        def kvref(j):
            return stg_s if isinstance(j, int) and j == 1 else kv_s.at[j]

        def qkv_store(j, qkv, t0, t1):
            for t in range(t0, t1):
                v = qkv[:, (t - t0) * 128:(t - t0 + 1) * 128]
                if t < 4 or t == 13:
                    v = v * (DH ** -0.5 * LOG2E)
                kvref(j)[t, HALO:HALO + TM, :] = v
                if t >= 4:
                    kvref(j + 1)[t, :HALO, :] = v[TM - HALO:]

        def qkv_dots(j, src, parts, n=None, kt=-1):
            k0, k1 = (0, 5) if n is None else (KCH[n][0], KCH[n][0] + 1)
            st = {}

            def mk(t0, t1):
                def dot(tief):
                    if 'h' not in st:
                        st['h'] = ld16(src, 0, TM, k0 * 128, k1 * 128)
                    st['h'] = tief(st['h'])
                    wq = ld16(wqt_s, t0 * 128, t1 * 128, k0 * 128, k1 * 128)
                    res = lax.dot_general(st['h'], wq, NT, preferred_element_type=f32)
                    acc = res if not n else res + part_s[j, :, t0 * 128:t1 * 128]
                    if n is not None and n < NK - 1:
                        part_s[j, :, t0 * 128:t1 * 128] = acc
                    else:
                        qkv_store(j, acc, t0, t1)
                    if t0 == kt:
                        ktl = lax.dot_general(ld16(wqt_s, 13 * 128, 13 * 128 + 64), st['h'], NT,
                                              preferred_element_type=f32)
                        qkv_store(j, jnp.concatenate([ktl, jnp.zeros((64, TM), f32)], axis=0).T, 13, 14)
                    return res
                return dot
            return [mk(*p) for p in parts]

        def attn_chunk(first, src, r, gate, jnext):
            r0 = r * RC
            q = [gated(src[t, HALO + r0:HALO + r0 + RC, :], gate) for t in Q_TILES]
            even = (lax.broadcasted_iota(jnp.int32, (RC, 128), 1) & 1) == 0
            ls = []
            for w in range(W):
                a = HALO + r0 - DIL * w
                p = q[0] * src[K_TILES[0], a:a + RC, :]
                for t in range(1, 5):
                    p = p + q[t] * src[K_TILES[t], a:a + RC, :]
                p = p + pltpu.roll(p, 64, 1)
                p = p + jnp.where(even, pltpu.roll(p, 127, 1), pltpu.roll(p, 1, 1))
                if first and r0 < DIL * w:
                    pos = r0 + lax.broadcasted_iota(jnp.int32, (RC, 128), 0)
                    p = jnp.where(pos >= DIL * w, p, -1e9 * LOG2E)
                ls.append(p)
            m = ls[0]
            for w in range(1, W):
                m = jnp.maximum(m, ls[w])
            es = [jnp.exp2(l - m) for l in ls]
            inv = 1.0 / _tree_sum(es)
            outs = []
            for t in range(5):
                acc = None
                for w in range(W):
                    a = HALO + r0 - DIL * w
                    term = es[w] * src[V_TILES[t], a:a + RC, :]
                    acc = term if acc is None else acc + term
                ob = (acc * inv).astype(bf16)
                outs.append(st16(o_s, r0, r0 + RC, slice(t * 128, (t + 1) * 128), ob))
            if jnext is None:
                return outs
            z = mkgate(outs)
            r1 = r0 + RC if r0 + RC < TM else TM + HALO
            for t in range(14):
                lo = max(r0, HALO) if t < 4 else r0
                if lo < r1:
                    v = gated(kv_s[jnext, t, lo:r1, :], z)
                    stg_s[t, lo:r1, :] = v
                    outs.append(v[:8])
            return outs

        def wo_dot(j):
            def dot(tief):
                attn_t = lax.dot_general(tief(ld16(wot_s, 0, D)), ld16(o_s, 0, TM), NT, preferred_element_type=f32)
                ga = jnp.concatenate([gcol_s[0]] * len(ALLC), axis=1)
                x1 = xt_s[j].astype(f32) + ga * attn_t
                x1n_s[...] = x1
                for c in ALLC:
                    ln2_stats[c] = ln_stats(lambda r, m: x1[r:r + m, c * 128:(c + 1) * 128], None)
                return attn_t
            return dot

        def wq_prep(k):
            r0, r1 = k * 128, min((k + 1) * 128, D)
            for s in range(14):
                if s < 13:
                    blk = wraw_s[r0:r1, s * 128:(s + 1) * 128]
                else:
                    blk = jnp.concatenate([wraw_s[r0:r1, s * 128:], jnp.zeros((r1 - r0, 64), bf16)], axis=1)
                if r1 - r0 < 128:
                    blk = jnp.concatenate([blk, jnp.zeros((128 - (r1 - r0), 128), bf16)], axis=0)
                tmp_s[k, s * 64:(s + 1) * 64, :] = pltpu.bitcast(blk.T, u32)
            for t in range(14):
                for g in range(2):
                    s0 = _pair_src(t, g)
                    if s0 >= 0:
                        wqt_s[t * 64 + g * 32:t * 64 + (g + 1) * 32, k * 128:(k + 1) * 128] = (
                            tmp_s[k, pl.ds(s0, H, stride=DH // 2), :])

        def wo_cvt(gate):
            outs = []
            for cc in range(5):
                if cc < 4:
                    v = wo_s[:, cc * 128:(cc + 1) * 128]
                else:
                    v = jnp.concatenate([wo_s[:, cc * 128:], jnp.zeros((D, 64), bf16)], axis=1)
                v = gated(pltpu.bitcast(v, u32), gate(cc * 48))
                tmp_s[cc, :D // 2, :] = v
                outs.append(v[D // 2 - 8:])
            return outs

        def wo_perm(t, gate):
            rows = []
            for g in range(2):
                s0 = _pair_src(V_TILES[t], g) - D
                if s0 >= 0:
                    rows.append(jnp.concatenate(
                        [gated(tmp_s[cc, pl.ds(s0, H, stride=DH // 2), :], gate) for cc in range(5)], axis=1))
                else:
                    rows.append(jnp.zeros((H, DP), u32))
            blk = pltpu.bitcast(jnp.concatenate(rows, axis=0), bf16).T[:D]
            bits = st16(wot_s, 0, D, slice(t * 128, (t + 1) * 128), blk)
            return [bits[k:k + 8] for k in (56, 120, 184, 248, 280)]

        def attn_task(first, src, r, jnext):
            return lambda gt: attn_chunk(first, src, r, gt(0), jnext)

        def ln1_task(j, dst, c):
            return lambda gt: ln1(j, dst, c, gt)

        def ident(h):
            return h

        start(g_first)
        start(g_second)
        for g in g_k:
            start(g)
        for jj in range(NLOOP):
            start(g_loop(jj))

        kv_s[0, 4:, :HALO, :] = jnp.zeros((10, HALO, 128), f32)
        zero_s[...] = jnp.zeros((8, 128), u32)
        wait(g_first)
        cvec = c_s[...].astype(f32)
        sc = (cvec * jax.nn.sigmoid(cvec)).astype(bf16)
        scol_s[...] = colbcast(padrow(sc.astype(f32)))

        st01, n01, mt = {}, {}, {}

        def norm_rows(j):
            for cc in ALLC:
                st01[j, cc] = ln_stats(xld(j, cc), None)
                n01[j, cc] = ln_norm(xld(j, cc), *st01[j, cc], KCH[0][0])

        def kprep(n, gate):
            k, mts = KCH[n]
            for t in mts:
                mt[t] = matvec(lambda r, m: wmod_s[r:r + m, t * 128:(t + 1) * 128], gate)
            sl = slice(k * 128, (k + 1) * 128)
            if k < 4:
                shift = mt[k]
                scale = 1.0 + jnp.concatenate([mt[4 + k][:, 64:], mt[5 + k][:, :64]], axis=1)
            else:
                z = jnp.zeros((1, 64), f32)
                shift = jnp.concatenate([mt[4][:, :64], z], axis=1)
                scale = jnp.concatenate([1.0 + mt[8][:, 64:], z], axis=1)
            mod_s[0, :, sl] = jnp.broadcast_to(scale, (8, 128))
            mod_s[1, :, sl] = jnp.broadcast_to(shift, (8, 128))
            for j, dst in ((0, ha_s), (1, hb_s)):
                for cc in ALLC:
                    v = n01[j, cc] if n == 0 else ln_norm(xld(j, cc), *st01[j, cc], k)
                    st16(dst, cc * 128, (cc + 1) * 128, sl, modulate(v, 0, sl))
            if n > 0:
                wq_prep(k)

        norm_rows(0)
        wait(g_second)
        wq_prep(KCH[0][0])
        norm_rows(1)
        for n in range(NK):
            wait(g_k[n])
            gate = None
            if n == 0:
                start(g_fin)
                start(g_gu)
                start(g_dn)
            else:
                gate = gates(qkv_dots(1, hb_s, ((sh, 12),), n - 1)[0](ident), 0)
            kprep(n, gate)
            if n < NK - 1:
                qkv_dots(0, ha_s, ((0, 12),), n)[0](ident)
                qkv_dots(1, hb_s, ((0, sh),), n)[0](ident)
        dots = (qkv_dots(0, ha_s, ((0, 12),), NK - 1) + qkv_dots(0, ha_s, ((12, 13),), kt=12)
                + qkv_dots(1, hb_s, ((12, 13),), kt=12) + qkv_dots(1, hb_s, ((0, 12),), NK - 1))
        run_slots(dots, [[(ln1_task(2, hc_s, 0), l1g[0]), (ln1_task(2, hc_s, 1), l1g[1])]], 2)

        def abody(jj, _):
            wait(g_loop(jj))

            def mod2_task(t):
                def task(gate):
                    v = matvec(lambda r, n: wm2_s[jj, r:r + n, t * 128:(t + 1) * 128], gate)
                    v = jnp.broadcast_to(v, (8, 128))
                    mraw_s[jj, :, t * 128:(t + 1) * 128] = v
                    return [v]
                return task
            tasks = dict(A=[ln1_task(3 + jj, hc_s, 0)], B=[ln1_task(3 + jj, hc_s, 1)],
                         m=[mod2_task(t) for t in range(MW // 128)])
            run_slots(qkv_dots(2 + jj, hc_s, QS, kt=kt_at[0]), parse_plan(lplan, tasks), lag[0])
            return 0
        lax.fori_loop(0, NLOOP, abody, 0)

        wait(g_fin)

        def mod_fin(gate):
            z = gate(0)
            mod = jnp.concatenate([gated(mraw_s[jj, :, t * 128:(t + 1) * 128], z)
                                   for jj in range(NLOOP) for t in range(MW // 128)], axis=1)
            mod_s[2] = padrow(0.5 + 0.5 * mod[:, 2 * D:3 * D])
            mod_s[3] = padrow(0.5 * mod[:, D:2 * D])
            ga = colbcast(padrow(mod[0:1, :D]))
            gb = colbcast(padrow(2.0 * mod[0:1, 3 * D:]))
            gcol_s[0] = ga
            gcol_s[1] = gb
            return [g[k:k + 8] for g in (ga, gb) for k in (120, 248, 376, 504, 568)]

        d7 = qkv_dots(7, ha_s, QS, kt=kt_at[3])
        dots = (qkv_dots(5, hc_s, QS, kt=kt_at[1]) + qkv_dots(6, hb_s, QS, kt=kt_at[2])
                + d7[:wpos] + [wo_dot(0)] + d7[wpos:])
        tasks = dict(A=[ln1_task(6, hb_s, 0)], B=[ln1_task(6, hb_s, 1)], C=[ln1_task(7, ha_s, 0)],
                     D=[ln1_task(7, ha_s, 1)], M=[mod_fin], V=[wo_cvt],
                     X=[lambda gt: ln2(0, gt)], Y=[lambda gt: ln2(1, gt)],
                     a=[attn_task(True, kv_s.at[0], r, None) for r in range(TM // RC)],
                     p=[(lambda gt, t=t: wo_perm(t, gt(0))) for t in range(5)])
        run_slots(dots, parse_plan(fplan, tasks), lag[1])
        wait(g_gu)

        def glu(g, u):
            return ((g * u) * (1.0 + jnp.tanh(g))).astype(bf16)

        def act_cols(rows, c0):
            h = pltpu.bitcast(h2n_s[rows, :D], bf16)
            last = glu(jnp.dot(h, w1_s[:, F - LC:], preferred_element_type=f32),
                       jnp.dot(h, w3_s[:, F - LC:], preferred_element_type=f32))
            return lambda: jnp.concatenate([pltpu.bitcast(act_s[rows, c0:], bf16), last], axis=1)

        def bbody(i, _):
            j2 = jnp.minimum(i + 2, NB - 1)
            st = {'h': ld16(h2n_s, 0, TM, 0, D)}

            def keep_x1(gate):
                outs = []
                for n, r in enumerate(range(0, D, 64)):
                    for c in ALLC:
                        v = gated(x1n_s[r:r + 64, c * 128:(c + 1) * 128], gate(n * gstep))
                        x1_s[r:r + 64, c * 128:(c + 1) * 128] = v
                        outs.append(v[56:])
                return outs

            def gdot(sl):
                def dot(tief):
                    st['h'] = tief(st['h'])
                    st['g'] = jnp.dot(st['h'], w1_s[:, sl], preferred_element_type=f32)
                    return st['g']
                return dot

            def udot(sl):
                def dot(tief):
                    st['h'] = tief(st['h'])
                    u = jnp.dot(st['h'], w3_s[:, sl], preferred_element_type=f32)
                    st16(act_s, 0, TM, sl, glu(st['g'], u))
                    return u
                return dot
            dots = []
            for c0 in range(0, F - LC, FC):
                sl = slice(c0, min(c0 + FC, F - LC))
                dots += [gdot(sl), udot(sl)]
            plan = [[(attn_task(False, stg_s, r, j2), 0)] for r in range(TM // RC)]
            plan[xpos[0]].append((keep_x1, xpos[1]))
            run_slots(dots, plan, lag[2])

            @pl.when(i == 0)
            def _():
                wait(g_dn)

            @pl.when(i < NB - 1)
            def _():
                KS = ks * 128
                tail = act_cols(slice(0, TM // 2), 2 * KS)
                wo_dot(i + 1)(ident)
                w = w2t_s[...]
                y0 = lax.dot_general(w[:, :KS], ld16(act_s, 0, TM, 0, KS), NT, preferred_element_type=f32)
                outs = ln2(0, gates(y0, 0)) + ln2(1, gates(y0, 1))
                y1 = lax.dot_general(w[:, KS:2 * KS], ld16(act_s, 0, TM, KS, 2 * KS), NT, preferred_element_type=f32)
                y2 = lax.dot_general(tie(w[:, 2 * KS:], mkgate(outs)), tail(), NT, preferred_element_type=f32)
                gb = jnp.concatenate([gcol_s[1]] * len(ALLC), axis=1)
                out_s[i] = (x1_s[...] + gb * (y0 + y1 + y2)).astype(bf16)
                cp(out_s.at[i], o_hbm.at[:, pl.ds(i * TM, TM)], osem).start()
            return 0
        lax.fori_loop(0, NB, bbody, 0)

        def qbody(c, _):
            cols = pl.ds(pl.multiple_of(c * 128, 128), 128)
            ocols = pl.ds(pl.multiple_of((NB - 1) * TM + c * 128, 128), 128)
            a = act_cols(pl.ds(pl.multiple_of(c * 64, 64), 64), 0)()
            y = lax.dot_general(w2t_s[...], a, NT, preferred_element_type=f32)
            for r0, r1 in zip(qsp[:-1], qsp[1:]):
                out_s[NB - 1, r0:r1, cols] = (x1_s[r0:r1, cols] + gcol_s[1, r0:r1, :] * y[r0:r1]).astype(bf16)
                cp(out_s.at[NB - 1, r0:r1, cols], o_hbm.at[r0:r1, ocols], osem).start()
            return 0
        lax.fori_loop(0, TM // 128, qbody, 0)
        cp(out_s, out_s, osem).wait()

    def fn(A_x, A_wqkv, A_wo, B_x, B_w1, B_w3, B_w2, c, w_mod):
        hbm = pl.BlockSpec(memory_space=pltpu.HBM)
        V = pltpu.VMEM
        rows16 = V((TM // 2, DP), u32)
        out_t = pl.pallas_call(
            kern,
            in_specs=[hbm] * 8,
            out_specs=hbm,
            out_shape=jax.ShapeDtypeStruct((D, S), bf16),
            scratch_shapes=[
                V((NB, D, TM), bf16), V((D, 3 * D), bf16), V((5, 14 * 64, 128), u32), V((14 * 64, DP), u32),
                V((D, D), bf16), V((D // 2, DP), u32), V((1, D), bf16), V((D, 2 * D), bf16),
                V((NLOOP, D, MW), bf16), V((NLOOP, 8, MW), f32),
                V((D, F), bf16), V((D, F), bf16), V((D, F), bf16),
                V((4, 8, DP), f32), V((2, D, 128), f32), V((D, 128), f32), V((2, TM, 12 * 128), f32),
                V((14, TM + HALO, 128), f32), V((NB + 1, 14, TM + HALO + pk, 128), f32),
                rows16, rows16, rows16, rows16, V((D, TM), f32), V((D, TM), f32), rows16,
                V((8, 128), u32), V((TM // 2, F - LC), u32), V((NB, D, TM), bf16),
                pltpu.SemaphoreType.DMA((NK + 2 + NLOOP,)),
            ],
            compiler_params=pltpu.CompilerParams(vmem_limit_bytes=110 * 1024 * 1024, disable_bounds_checks=True),
        )(A_x[0].T, A_wqkv, A_wo, B_w1, B_w3, B_w2.T, c, w_mod)
        return out_t.T[None]
    return fn


_impl = make()


@jax.jit
def pallas_adaLN_cond__sliding_local_dilated__glu_gated_swiglu__prompt_kernel(
    A_x: jax.Array,
    A_wqkv: jax.Array,
    A_wo: jax.Array,
    B_x: jax.Array,
    B_w1: jax.Array,
    B_w3: jax.Array,
    B_w2: jax.Array,
    c: jax.Array,
    w_mod: jax.Array,
):
    return _impl(A_x, A_wqkv, A_wo, B_x, B_w1, B_w3, B_w2, c, w_mod)
```

```python
import math

import jax
import jax.numpy as jnp
from jax import lax
from jax.experimental import pallas as pl
from jax.experimental.pallas import tpu as pltpu

S, D, F = 2048, 576, 4608
H, DH, W, DIL = 32, 18, 8, 2
DP = 640
NT = (((1,), (1,)), ((), ()))
f32, bf16, u32 = jnp.float32, jnp.bfloat16, jnp.uint32
LOG2E = math.log2(math.e)
EPS = 1e-5
HALO = 16
TM = 256
RC = 16
FC = 512
LC = 256
NB = S // TM
NLOOP = 3
MW = 4 * D // NLOOP


def _pair_src(t, g):
    if t < 12:
        return (t // 4) * (D // 2) + 2 * (t % 4) + g
    if t == 12:
        return 8 if g == 0 else D + 8
    return D // 2 + 8 if g == 0 else -1


Q_TILES = (0, 1, 2, 3, 12)
K_TILES = (4, 5, 6, 7, 13)
V_TILES = (8, 9, 10, 11, 12)
KCH = ((4, (4, 8)), (0, (0, 5)), (1, (1, 6)), (2, (2, 7)), (3, (3,)))
NK = len(KCH)


def _tree_sum(parts):
    while len(parts) > 1:
        parts = [parts[k] + parts[k + 1] if k + 1 < len(parts) else parts[k] for k in range(0, len(parts), 2)]
    return parts[0]


def make(QS=((4, 8), (0, 4), (8, 11), (11, 13)), kt_at=(8, 4, 11, 4), lag=(1, 2, 1), gstep=24, ks=4, pk=8,
         l1g=(0, 4, 8), qsp=(0, 256, 448, 576), xpos=(0, 2), wpos=2, lplan='A,m,m,m|B,m,m,m',
         fplan='V,A,a,a|p,B,a,.|a,M,a|p,a|a,C,.,.|D,a,p,a|a,a,a|p,p|a,a,a,a|.|.|X,.,Y'):

    def kern(xt_hbm, wqkv_hbm, wo_hbm, w1_hbm, w3_hbm, w2t_hbm, c_hbm, wmod_hbm, o_hbm,
             xt_s, wraw_s, tmp_s, wqt_s, wqn_s, wo_s, wot_s, c_s, wmod_s, wm2_s, mraw_s, w1_s, w3_s, w2t_s,
             mod_s, gcol_s, scol_s, part_s, stg_s, kv_s, ha_s, hb_s, hc_s, o_s, x1_s, x1n_s, h2n_s,
             zero_s, act_s, out_s, sems):
        cp = pltpu.make_async_copy

        def x_copy(j, sem):
            return cp(xt_hbm.at[:, pl.ds(j * TM, TM)], xt_s.at[j], sems.at[sem])

        def wq_copy(k, sem):
            rows = slice(k * 128, min((k + 1) * 128, D))
            return cp(wqkv_hbm.at[rows, :], wraw_s.at[rows, :], sems.at[sem])

        g_first = [x_copy(0, 0), cp(c_hbm, c_s, sems.at[0])]
        g_second = [x_copy(1, 1), wq_copy(KCH[0][0], 1)]
        g_k = []
        for n, (k, mts) in enumerate(KCH):
            g = [cp(wmod_hbm.at[:, t * 128:(t + 1) * 128], wmod_s.at[:, t * 128:(t + 1) * 128], sems.at[2 + n])
                 for t in mts]
            if n > 0:
                g.append(wq_copy(k, 2 + n))
            g_k.append(g)
        g_k[NK - 1].append(x_copy(2, NK + 1))

        def g_loop(jj):
            cols = pl.ds(pl.multiple_of(2 * D + jj * MW, 128), MW)
            return [x_copy(3 + jj, NK + 2 + jj), cp(wmod_hbm.at[:, cols], wm2_s.at[jj], sems.at[NK + 2 + jj])]

        g_fin = [x_copy(j, 0) for j in range(3 + NLOOP, NB)] + [cp(wo_hbm, wo_s, sems.at[0])]
        g_gu = [cp(w1_hbm, w1_s, sems.at[1]), cp(w3_hbm, w3_s, sems.at[1])]
        g_dn = [cp(w2t_hbm, w2t_s, sems.at[2])]
        osem = sems.at[3]

        def start(g):
            for c in g:
                c.start()

        def wait(g):
            for c in g:
                c.wait()

        def ld16(ref, r0, r1, c0=0, c1=None):
            return pltpu.bitcast(ref[r0 // 2:r1 // 2, c0:c1], bf16)

        def st16(ref, r0, r1, sl, v):
            bits = pltpu.bitcast(v, u32)
            ref[r0 // 2:r1 // 2, sl] = bits
            return bits

        def gated(v, gate):
            if gate is None:
                return v
            bits = pltpu.bitcast(v, u32) if v.dtype != u32 else v
            z = gate if bits.shape[0] == 8 else jnp.concatenate([gate] * (bits.shape[0] // 8), axis=0)
            return pltpu.bitcast(bits | z, v.dtype) if v.dtype != u32 else bits | z

        def mkgate(outs):
            z = None
            for ob in outs:
                bb = ob if ob.dtype == u32 else pltpu.bitcast(ob, u32)
                z = bb if z is None else z | bb
            return z & zero_s[...]

        def tie(h, z):
            if z is None:
                return h
            top = gated(h[:16, :128], z)
            if h.shape[1] > 128:
                top = jnp.concatenate([top, h[:16, 128:]], axis=1)
            return jnp.concatenate([top, h[16:]], axis=0)

        def gates(res, t):
            return lambda r: mkgate([res[r:r + 8, t * 128:(t + 1) * 128]])

        def run_slots(dots, plan, lag):
            pend = []
            for k, dot in enumerate(dots):
                z = pend.pop(0) if len(pend) > lag else None
                res = dot(lambda h: tie(h, z))
                new = []
                for task, t in (plan[k] if k < len(plan) else []):
                    new += task(gates(res, t))
                pend.append(mkgate(new) if new else None)

        def parse_plan(text, tasks):
            plan = []
            for slot in text.split('|'):
                row = []
                for t, names in enumerate(slot.split(',')):
                    for ch in names.strip('.'):
                        row.append((tasks[ch].pop(0), t))
                plan.append(row)
            assert not any(tasks.values())
            return plan

        def rowsum(a):
            return jnp.sum(_tree_sum([a[k:k + 8] for k in range(0, a.shape[0], 8)]), axis=0, keepdims=True)

        def ln_stats(ld, gate):
            piv = ld(0, 8)[0:1]
            piv8 = jnp.broadcast_to(piv, (8, 128))
            a1 = a2 = None
            for n, r in enumerate(range(0, D, 64)):
                p = piv if gate is None else gated(piv8, gate(n * gstep))[0:1]
                v = ld(r, 64) - p
                v1 = v[:32] + v[32:]
                v = v * v
                v2 = v[:32] + v[32:]
                a1 = v1 if a1 is None else a1 + v1
                a2 = v2 if a2 is None else a2 + v2
            s1, s2 = rowsum(a1) * (1.0 / D), rowsum(a2) * (1.0 / D)
            var = jnp.maximum(s2 - s1 * s1, 0.0)
            return piv + s1, lax.rsqrt(var + EPS)

        def ln_norm(ld, m, rstd, t):
            n = min(128, D - t * 128)
            blk = (ld(t * 128, n) - m) * rstd
            if n < 128:
                blk = jnp.concatenate([blk, jnp.zeros((128 - n, 128), f32)], axis=0)
            return blk.T

        def modulate(v, k, sl):
            return (v * mod_s[2 * k, 0:1, sl] + mod_s[2 * k + 1, 0:1, sl]).astype(bf16)

        def ln_apply(ld, m, rstd, k, dst, c):
            outs = []
            for t in range(5):
                sl = slice(t * 128, (t + 1) * 128)
                hb = modulate(ln_norm(ld, m, rstd, t), k, sl)
                outs.append(st16(dst, c * 128, (c + 1) * 128, sl, hb)[56:])
            return outs

        ALLC = tuple(range(TM // 128))
        ln2_stats = {}

        def xld(j, c):
            return lambda r, n: xt_s[j, r:r + n, c * 128:(c + 1) * 128].astype(f32)

        def ln1(j, dst, c, gate):
            ld = xld(j, c)
            return ln_apply(ld, *ln_stats(ld, gate), 0, dst, c)

        def ln2(c, gate):
            m, rstd = ln2_stats[c]
            m = gated(jnp.broadcast_to(m, (8, 128)), gate(0))[0:1]
            return ln_apply(lambda r, n: x1n_s[r:r + n, c * 128:(c + 1) * 128], m, rstd, 1, h2n_s, c)

        def padrow(r):
            return jnp.concatenate([r, jnp.zeros((r.shape[0], DP - D), f32)], axis=1)

        def colbcast(row):
            return jnp.broadcast_to(row, (128, DP)).T[:D]

        def matvec(ld, gate):
            acc = None
            for n, r in enumerate(range(0, D, 64)):
                sv = scol_s[r:r + 64, :]
                if gate is not None:
                    sv = gated(sv, gate(n * gstep))
                v = ld(r, 64).astype(f32) * sv
                v = v[:32] + v[32:]
                acc = v if acc is None else acc + v
            return rowsum(acc)

        def kvref(j):
            return stg_s if isinstance(j, int) and j == 1 else kv_s.at[j]

        def qkv_store(j, qkv, t0, t1):
            for t in range(t0, t1):
                v = qkv[:, (t - t0) * 128:(t - t0 + 1) * 128]
                if t < 4 or t == 13:
                    v = v * (DH ** -0.5 * LOG2E)
                kvref(j)[t, HALO:HALO + TM, :] = v
                if t >= 4:
                    kvref(j + 1)[t, :HALO, :] = v[TM - HALO:]

        def qkv_dots(j, src, parts, n=None, kt=-1):
            k0, k1 = (0, 5) if n is None else (KCH[n][0], KCH[n][0] + 1)
            st = {}

            def mk(t0, t1):
                def dot(tief):
                    if 'h' not in st:
                        st['h'] = ld16(src, 0, TM, k0 * 128, k1 * 128)
                    st['h'] = tief(st['h'])
                    if (t0, t1) == (4, 8):
                        res = jnp.dot(st['h'], ld16(wqn_s, k0 * 128, k1 * 128), preferred_element_type=f32)
                    else:
                        wq = ld16(wqt_s, t0 * 128, t1 * 128, k0 * 128, k1 * 128)
                        res = lax.dot_general(st['h'], wq, NT, preferred_element_type=f32)
                    acc = res if not n else res + part_s[j, :, t0 * 128:t1 * 128]
                    if n is not None and n < NK - 1:
                        part_s[j, :, t0 * 128:t1 * 128] = acc
                    else:
                        qkv_store(j, acc, t0, t1)
                    if t0 == kt:
                        ktl = lax.dot_general(ld16(wqt_s, 13 * 128, 13 * 128 + 64), st['h'], NT,
                                              preferred_element_type=f32)
                        qkv_store(j, jnp.concatenate([ktl, jnp.zeros((64, TM), f32)], axis=0).T, 13, 14)
                    return res
                return dot
            return [mk(*p) for p in parts]

        def attn_chunk(first, src, r, gate, jnext):
            r0 = r * RC
            q = [gated(src[t, HALO + r0:HALO + r0 + RC, :], gate) for t in Q_TILES]
            even = (lax.broadcasted_iota(jnp.int32, (RC, 128), 1) & 1) == 0
            ls = []
            for w in range(W):
                a = HALO + r0 - DIL * w
                p = q[0] * src[K_TILES[0], a:a + RC, :]
                for t in range(1, 5):
                    p = p + q[t] * src[K_TILES[t], a:a + RC, :]
                p = p + pltpu.roll(p, 64, 1)
                p = p + jnp.where(even, pltpu.roll(p, 127, 1), pltpu.roll(p, 1, 1))
                if first and r0 < DIL * w:
                    pos = r0 + lax.broadcasted_iota(jnp.int32, (RC, 128), 0)
                    p = jnp.where(pos >= DIL * w, p, -1e9 * LOG2E)
                ls.append(p)
            m = ls[0]
            for w in range(1, W):
                m = jnp.maximum(m, ls[w])
            es = [jnp.exp2(l - m) for l in ls]
            inv = 1.0 / _tree_sum(es)
            outs = []
            for t in range(5):
                acc = None
                for w in range(W):
                    a = HALO + r0 - DIL * w
                    term = es[w] * src[V_TILES[t], a:a + RC, :]
                    acc = term if acc is None else acc + term
                ob = (acc * inv).astype(bf16)
                outs.append(st16(o_s, r0, r0 + RC, slice(t * 128, (t + 1) * 128), ob))
            if jnext is None:
                return outs
            z = mkgate(outs)
            r1 = r0 + RC if r0 + RC < TM else TM + HALO
            for t in range(14):
                lo = max(r0, HALO) if t < 4 else r0
                if lo < r1:
                    v = gated(kv_s[jnext, t, lo:r1, :], z)
                    stg_s[t, lo:r1, :] = v
                    outs.append(v[:8])
            return outs

        def wo_dot(j):
            def dot(tief):
                attn_t = lax.dot_general(tief(ld16(wot_s, 0, D)), ld16(o_s, 0, TM), NT, preferred_element_type=f32)
                ga = jnp.concatenate([gcol_s[0]] * len(ALLC), axis=1)
                x1 = xt_s[j].astype(f32) + ga * attn_t
                x1n_s[...] = x1
                for c in ALLC:
                    ln2_stats[c] = ln_stats(lambda r, m: x1[r:r + m, c * 128:(c + 1) * 128], None)
                return attn_t
            return dot

        def wq_prep(k):
            r0, r1 = k * 128, min((k + 1) * 128, D)
            for s in range(14):
                if s < 13:
                    blk = wraw_s[r0:r1, s * 128:(s + 1) * 128]
                else:
                    blk = jnp.concatenate([wraw_s[r0:r1, s * 128:], jnp.zeros((r1 - r0, 64), bf16)], axis=1)
                if r1 - r0 < 128:
                    blk = jnp.concatenate([blk, jnp.zeros((128 - (r1 - r0), 128), bf16)], axis=0)
                tmp_s[k, s * 64:(s + 1) * 64, :] = pltpu.bitcast(blk.T, u32)
            for t in range(14):
                rows = [tmp_s[k, pl.ds(_pair_src(t, g), H, stride=DH // 2), :] for g in range(2) if _pair_src(t, g) >= 0]
                rows = jnp.concatenate(rows, axis=0)
                wqt_s[t * 64:t * 64 + rows.shape[0], k * 128:(k + 1) * 128] = rows

        def wq_untr(k, gate):
            outs = []
            for t in range(4, 8):
                rows = gated(wqt_s[t * 64:(t + 1) * 64, k * 128:(k + 1) * 128], gate)
                bits = st16(wqn_s, k * 128, (k + 1) * 128, slice((t - 4) * 128, (t - 3) * 128), pltpu.bitcast(rows, bf16).T)
                outs.append(bits[56:])
            return outs

        def wo_cvt(gate):
            outs = []
            for cc in range(5):
                if cc < 4:
                    v = wo_s[:, cc * 128:(cc + 1) * 128]
                else:
                    v = jnp.concatenate([wo_s[:, cc * 128:], jnp.zeros((D, 64), bf16)], axis=1)
                v = gated(pltpu.bitcast(v, u32), gate(cc * 48))
                tmp_s[cc, :D // 2, :] = v
                outs.append(v[D // 2 - 8:])
            return outs

        def wo_perm(t, gate):
            rows = []
            for g in range(2):
                s0 = _pair_src(V_TILES[t], g) - D
                if s0 >= 0:
                    rows.append(jnp.concatenate(
                        [gated(tmp_s[cc, pl.ds(s0, H, stride=DH // 2), :], gate) for cc in range(5)], axis=1))
                else:
                    rows.append(jnp.zeros((H, DP), u32))
            blk = pltpu.bitcast(jnp.concatenate(rows, axis=0), bf16).T[:D]
            bits = st16(wot_s, 0, D, slice(t * 128, (t + 1) * 128), blk)
            return [bits[k:k + 8] for k in (56, 120, 184, 248, 280)]

        def attn_task(first, src, r, jnext):
            return lambda gt: attn_chunk(first, src, r, gt(0), jnext)

        def ln1_task(j, dst, c):
            return lambda gt: ln1(j, dst, c, gt)

        def untr_task(k):
            return lambda gt: wq_untr(k, gt(0))

        def ident(h):
            return h

        start(g_first)
        start(g_second)
        for g in g_k:
            start(g)
        for jj in range(NLOOP):
            start(g_loop(jj))

        kv_s[0, 4:, :HALO, :] = jnp.zeros((10, HALO, 128), f32)
        zero_s[...] = jnp.zeros((8, 128), u32)
        wait(g_first)
        cvec = c_s[...].astype(f32)
        sc = (cvec * jax.nn.sigmoid(cvec)).astype(bf16)
        scol_s[...] = colbcast(padrow(sc.astype(f32)))

        st01, n01, mt = {}, {}, {}

        def norm_rows(j):
            for cc in ALLC:
                st01[j, cc] = ln_stats(xld(j, cc), None)
                n01[j, cc] = ln_norm(xld(j, cc), *st01[j, cc], KCH[0][0])

        def kprep(n, gate):
            k, mts = KCH[n]
            for t in mts:
                mt[t] = matvec(lambda r, m: wmod_s[r:r + m, t * 128:(t + 1) * 128], gate)
            sl = slice(k * 128, (k + 1) * 128)
            if k < 4:
                shift = mt[k]
                scale = 1.0 + jnp.concatenate([mt[4 + k][:, 64:], mt[5 + k][:, :64]], axis=1)
            else:
                z = jnp.zeros((1, 64), f32)
                shift = jnp.concatenate([mt[4][:, :64], z], axis=1)
                scale = jnp.concatenate([1.0 + mt[8][:, 64:], z], axis=1)
            mod_s[0, :, sl] = jnp.broadcast_to(scale, (8, 128))
            mod_s[1, :, sl] = jnp.broadcast_to(shift, (8, 128))
            for j, dst in ((0, ha_s), (1, hb_s)):
                for cc in ALLC:
                    v = n01[j, cc] if n == 0 else ln_norm(xld(j, cc), *st01[j, cc], k)
                    st16(dst, cc * 128, (cc + 1) * 128, sl, modulate(v, 0, sl))
            if n > 0:
                wq_prep(k)

        norm_rows(0)
        wait(g_second)
        wq_prep(KCH[0][0])
        norm_rows(1)
        for n in range(NK):
            wait(g_k[n])
            gate = None
            if n == 0:
                start(g_fin)
                start(g_gu)
                start(g_dn)
            else:
                gate = gates([d(ident) for d in qkv_dots(1, hb_s, ((4, 8), (8, 12)), n - 1)][0], 0)
            kprep(n, gate)
            if n < NK - 1:
                dots = qkv_dots(0, ha_s, ((0, 12),), n) + qkv_dots(1, hb_s, ((0, 4),), n)
                run_slots(dots, [[(untr_task(KCH[n][0]), 0)]], 0)
        dots = (qkv_dots(0, ha_s, ((0, 12),), NK - 1) + qkv_dots(0, ha_s, ((12, 13),), kt=12)
                + qkv_dots(1, hb_s, ((12, 13),), kt=12) + qkv_dots(1, hb_s, ((0, 12),), NK - 1))
        run_slots(dots, [[(ln1_task(2, hc_s, 0), l1g[0]), (ln1_task(2, hc_s, 1), l1g[1]), (untr_task(KCH[NK - 1][0]), l1g[2])]], 2)

        def abody(jj, _):
            wait(g_loop(jj))

            def mod2_task(t):
                def task(gate):
                    v = matvec(lambda r, n: wm2_s[jj, r:r + n, t * 128:(t + 1) * 128], gate)
                    v = jnp.broadcast_to(v, (8, 128))
                    mraw_s[jj, :, t * 128:(t + 1) * 128] = v
                    return [v]
                return task
            tasks = dict(A=[ln1_task(3 + jj, hc_s, 0)], B=[ln1_task(3 + jj, hc_s, 1)],
                         m=[mod2_task(t) for t in range(MW // 128)])
            run_slots(qkv_dots(2 + jj, hc_s, QS, kt=kt_at[0]), parse_plan(lplan, tasks), lag[0])
            return 0
        lax.fori_loop(0, NLOOP, abody, 0)

        wait(g_fin)

        def mod_fin(gate):
            z = gate(0)
            mod = jnp.concatenate([gated(mraw_s[jj, :, t * 128:(t + 1) * 128], z)
                                   for jj in range(NLOOP) for t in range(MW // 128)], axis=1)
            mod_s[2] = padrow(0.5 + 0.5 * mod[:, 2 * D:3 * D])
            mod_s[3] = padrow(0.5 * mod[:, D:2 * D])
            ga = colbcast(padrow(mod[0:1, :D]))
            gb = colbcast(padrow(2.0 * mod[0:1, 3 * D:]))
            gcol_s[0] = ga
            gcol_s[1] = gb
            return [g[k:k + 8] for g in (ga, gb) for k in (120, 248, 376, 504, 568)]

        d7 = qkv_dots(7, ha_s, QS, kt=kt_at[3])
        dots = (qkv_dots(5, hc_s, QS, kt=kt_at[1]) + qkv_dots(6, hb_s, QS, kt=kt_at[2])
                + d7[:wpos] + [wo_dot(0)] + d7[wpos:])
        tasks = dict(A=[ln1_task(6, hb_s, 0)], B=[ln1_task(6, hb_s, 1)], C=[ln1_task(7, ha_s, 0)],
                     D=[ln1_task(7, ha_s, 1)], M=[mod_fin], V=[wo_cvt],
                     X=[lambda gt: ln2(0, gt)], Y=[lambda gt: ln2(1, gt)],
                     a=[attn_task(True, kv_s.at[0], r, None) for r in range(TM // RC)],
                     p=[(lambda gt, t=t: wo_perm(t, gt(0))) for t in range(5)])
        run_slots(dots, parse_plan(fplan, tasks), lag[1])
        wait(g_gu)

        def glu(g, u):
            return ((g * u) * (1.0 + jnp.tanh(g))).astype(bf16)

        def act_cols(rows, c0):
            h = pltpu.bitcast(h2n_s[rows, :D], bf16)
            last = glu(jnp.dot(h, w1_s[:, F - LC:], preferred_element_type=f32),
                       jnp.dot(h, w3_s[:, F - LC:], preferred_element_type=f32))
            return lambda: jnp.concatenate([pltpu.bitcast(act_s[rows, c0:], bf16), last], axis=1)

        def bbody(i, _):
            j2 = jnp.minimum(i + 2, NB - 1)
            st = {'h': ld16(h2n_s, 0, TM, 0, D)}

            def keep_x1(gate):
                outs = []
                for n, r in enumerate(range(0, D, 64)):
                    for c in ALLC:
                        v = gated(x1n_s[r:r + 64, c * 128:(c + 1) * 128], gate(n * gstep))
                        x1_s[r:r + 64, c * 128:(c + 1) * 128] = v
                        outs.append(v[56:])
                return outs

            def gdot(sl):
                def dot(tief):
                    st['h'] = tief(st['h'])
                    st['g'] = jnp.dot(st['h'], w1_s[:, sl], preferred_element_type=f32)
                    return st['g']
                return dot

            def udot(sl):
                def dot(tief):
                    st['h'] = tief(st['h'])
                    u = jnp.dot(st['h'], w3_s[:, sl], preferred_element_type=f32)
                    st16(act_s, 0, TM, sl, glu(st['g'], u))
                    return u
                return dot
            dots = []
            for c0 in range(0, F - LC, FC):
                sl = slice(c0, min(c0 + FC, F - LC))
                dots += [gdot(sl), udot(sl)]
            plan = [[(attn_task(False, stg_s, r, j2), 0)] for r in range(TM // RC)]
            plan[xpos[0]].append((keep_x1, xpos[1]))
            run_slots(dots, plan, lag[2])

            @pl.when(i == 0)
            def _():
                wait(g_dn)

            @pl.when(i < NB - 1)
            def _():
                KS = ks * 128
                tail = act_cols(slice(0, TM // 2), 2 * KS)
                wo_dot(i + 1)(ident)
                w = w2t_s[...]
                y0 = lax.dot_general(w[:, :KS], ld16(act_s, 0, TM, 0, KS), NT, preferred_element_type=f32)
                outs = ln2(0, gates(y0, 0)) + ln2(1, gates(y0, 1))
                y1 = lax.dot_general(w[:, KS:2 * KS], ld16(act_s, 0, TM, KS, 2 * KS), NT, preferred_element_type=f32)
                y2 = lax.dot_general(tie(w[:, 2 * KS:], mkgate(outs)), tail(), NT, preferred_element_type=f32)
                gb = jnp.concatenate([gcol_s[1]] * len(ALLC), axis=1)
                out_s[i] = (x1_s[...] + gb * (y0 + y1 + y2)).astype(bf16)
                cp(out_s.at[i], o_hbm.at[:, pl.ds(i * TM, TM)], osem).start()
            return 0
        lax.fori_loop(0, NB, bbody, 0)

        def qbody(c, _):
            cols = pl.ds(pl.multiple_of(c * 128, 128), 128)
            ocols = pl.ds(pl.multiple_of((NB - 1) * TM + c * 128, 128), 128)
            a = act_cols(pl.ds(pl.multiple_of(c * 64, 64), 64), 0)()
            y = lax.dot_general(w2t_s[...], a, NT, preferred_element_type=f32)
            for r0, r1 in zip(qsp[:-1], qsp[1:]):
                out_s[NB - 1, r0:r1, cols] = (x1_s[r0:r1, cols] + gcol_s[1, r0:r1, :] * y[r0:r1]).astype(bf16)
                cp(out_s.at[NB - 1, r0:r1, cols], o_hbm.at[r0:r1, ocols], osem).start()
            return 0
        lax.fori_loop(0, TM // 128, qbody, 0)
        cp(o_hbm, o_hbm, osem).wait()

    def fn(A_x, A_wqkv, A_wo, B_x, B_w1, B_w3, B_w2, c, w_mod):
        hbm = pl.BlockSpec(memory_space=pltpu.HBM)
        V = pltpu.VMEM
        rows16 = V((TM // 2, DP), u32)
        out_t = pl.pallas_call(
            kern,
            in_specs=[hbm] * 8,
            out_specs=hbm,
            out_shape=jax.ShapeDtypeStruct((D, S), bf16),
            scratch_shapes=[
                V((NB, D, TM), bf16), V((D, 3 * D), bf16), V((5, 14 * 64, 128), u32), V((14 * 64, DP), u32), V((DP // 2, 512), u32),
                V((D, D), bf16), V((D // 2, DP), u32), V((1, D), bf16), V((D, 2 * D), bf16),
                V((NLOOP, D, MW), bf16), V((NLOOP, 8, MW), f32),
                V((D, F), bf16), V((D, F), bf16), V((D, F), bf16),
                V((4, 8, DP), f32), V((2, D, 128), f32), V((D, 128), f32), V((2, TM, 12 * 128), f32),
                V((14, TM + HALO, 128), f32), V((NB + 1, 14, TM + HALO + pk, 128), f32),
                rows16, rows16, rows16, rows16, V((D, TM), f32), V((D, TM), f32), rows16,
                V((8, 128), u32), V((TM // 2, F - LC), u32), V((NB, D, TM), bf16),
                pltpu.SemaphoreType.DMA((NK + 2 + NLOOP,)),
            ],
            compiler_params=pltpu.CompilerParams(vmem_limit_bytes=110 * 1024 * 1024, disable_bounds_checks=True),
        )(A_x[0].T, A_wqkv, A_wo, B_w1, B_w3, B_w2.T, c, w_mod)
        return out_t.T[None]
    return fn


_impl = make()


@jax.jit
def pallas_adaLN_cond__sliding_local_dilated__glu_gated_swiglu__prompt_kernel(
    A_x: jax.Array,
    A_wqkv: jax.Array,
    A_wo: jax.Array,
    B_x: jax.Array,
    B_w1: jax.Array,
    B_w3: jax.Array,
    B_w2: jax.Array,
    c: jax.Array,
    w_mod: jax.Array,
):
    return _impl(A_x, A_wqkv, A_wo, B_x, B_w1, B_w3, B_w2, c, w_mod)
```

```python
import math

import jax
import jax.numpy as jnp
from jax import lax
from jax.experimental import pallas as pl
from jax.experimental.pallas import tpu as pltpu

S, D, F = 2048, 576, 4608
H, DH, W, DIL = 32, 18, 8, 2
DP = 640
NT = (((1,), (1,)), ((), ()))
f32, bf16, u32 = jnp.float32, jnp.bfloat16, jnp.uint32
LOG2E = math.log2(math.e)
EPS = 1e-5
HALO = 16
TM = 256
RC = 16
FC = 512
LC = 256
NB = S // TM
NLOOP = 3
MW = 4 * D // NLOOP


def _pair_src(t, g):
    if t < 12:
        return (t // 4) * (D // 2) + 2 * (t % 4) + g
    if t == 12:
        return 8 if g == 0 else D + 8
    return D // 2 + 8 if g == 0 else -1


Q_TILES = (0, 1, 2, 3, 12)
K_TILES = (4, 5, 6, 7, 13)
V_TILES = (8, 9, 10, 11, 12)
KCH = ((4, (4, 8)), (0, (0, 5)), (1, (1, 6)), (2, (2, 7)), (3, (3,)))
NK = len(KCH)


def _tree_sum(parts):
    while len(parts) > 1:
        parts = [parts[k] + parts[k + 1] if k + 1 < len(parts) else parts[k] for k in range(0, len(parts), 2)]
    return parts[0]


def make(QS=((4, 8), (0, 4), (8, 11), (11, 13)), kt_at=(8, 4, 11, 4), lag=(1, 2, 1), gstep=24, ks=4, pk=8,
         l1g=(0, 4, 8), qsp=(0, 256, 448, 576), xpos=(0, 2), wpos=2, lplan='A,m,m,m|B,m,m,m',
         fplan='V,A,a,a|p,B,a,.|a,M,a|p,a|a,C,.,.|D,a,p,a|a,a,a|p,p|a,a,a,a|.|.|X,.,Y'):

    def kern(xt_hbm, wqkv_hbm, wo_hbm, w1_hbm, w3_hbm, w2t_hbm, c_hbm, wmod_hbm, o_hbm,
             xt_s, wraw_s, tmp_s, wqt_s, wqn_s, wo_s, wot_s, c_s, wmod_s, wm2_s, mraw_s, w1_s, w3_s, w2t_s,
             mod_s, gcol_s, scol_s, part_s, stg_s, kv_s, ha_s, hb_s, hc_s, o_s, x1_s, x1n_s, h2n_s,
             zero_s, act_s, out_s, sems):
        cp = pltpu.make_async_copy

        def x_copy(j, sem):
            return cp(xt_hbm.at[:, pl.ds(j * TM, TM)], xt_s.at[j], sems.at[sem])

        def wq_copy(k, sem):
            rows = slice(k * 128, min((k + 1) * 128, D))
            return cp(wqkv_hbm.at[rows, :], wraw_s.at[rows, :], sems.at[sem])

        g_first = [x_copy(0, 0), cp(c_hbm, c_s, sems.at[0])]
        g_second = [x_copy(1, 1)]
        g_k = []
        for n, (k, mts) in enumerate(KCH):
            g = [cp(wmod_hbm.at[:, t * 128:(t + 1) * 128], wmod_s.at[:, t * 128:(t + 1) * 128], sems.at[2 + n])
                 for t in mts]
            g.append(wq_copy(k, 2 + n))
            g_k.append(g)
        g_k[NK - 1].append(x_copy(2, NK + 1))

        def g_loop(jj):
            cols = pl.ds(pl.multiple_of(2 * D + jj * MW, 128), MW)
            return [x_copy(3 + jj, NK + 2 + jj), cp(wmod_hbm.at[:, cols], wm2_s.at[jj], sems.at[NK + 2 + jj])]

        g_fin = [x_copy(j, 0) for j in range(3 + NLOOP, NB)] + [cp(wo_hbm, wo_s, sems.at[0])]
        g_gu = [cp(w1_hbm, w1_s, sems.at[1]), cp(w3_hbm, w3_s, sems.at[1])]
        g_dn = [cp(w2t_hbm, w2t_s, sems.at[2])]
        osem = sems.at[3]

        def start(g):
            for c in g:
                c.start()

        def wait(g):
            for c in g:
                c.wait()

        def ld16(ref, r0, r1, c0=0, c1=None):
            return pltpu.bitcast(ref[r0 // 2:r1 // 2, c0:c1], bf16)

        def st16(ref, r0, r1, sl, v):
            bits = pltpu.bitcast(v, u32)
            ref[r0 // 2:r1 // 2, sl] = bits
            return bits

        def gated(v, gate):
            if gate is None:
                return v
            bits = pltpu.bitcast(v, u32) if v.dtype != u32 else v
            z = gate if bits.shape[0] == 8 else jnp.concatenate([gate] * (bits.shape[0] // 8), axis=0)
            return pltpu.bitcast(bits | z, v.dtype) if v.dtype != u32 else bits | z

        def mkgate(outs):
            z = None
            for ob in outs:
                bb = ob if ob.dtype == u32 else pltpu.bitcast(ob, u32)
                z = bb if z is None else z | bb
            return z & zero_s[...]

        def tie(h, z):
            if z is None:
                return h
            top = gated(h[:16, :128], z)
            if h.shape[1] > 128:
                top = jnp.concatenate([top, h[:16, 128:]], axis=1)
            return jnp.concatenate([top, h[16:]], axis=0)

        def gates(res, t):
            return lambda r: mkgate([res[r:r + 8, t * 128:(t + 1) * 128]])

        def run_slots(dots, plan, lag):
            pend = []
            for k, dot in enumerate(dots):
                z = pend.pop(0) if len(pend) > lag else None
                res = dot(lambda h: tie(h, z))
                new = []
                for task, t in (plan[k] if k < len(plan) else []):
                    new += task(gates(res, t))
                pend.append(mkgate(new) if new else None)

        def parse_plan(text, tasks):
            plan = []
            for slot in text.split('|'):
                row = []
                for t, names in enumerate(slot.split(',')):
                    for ch in names.strip('.'):
                        row.append((tasks[ch].pop(0), t))
                plan.append(row)
            assert not any(tasks.values())
            return plan

        def rowsum(a):
            return jnp.sum(_tree_sum([a[k:k + 8] for k in range(0, a.shape[0], 8)]), axis=0, keepdims=True)

        def ln_stats(ld, gate):
            piv = ld(0, 8)[0:1]
            piv8 = jnp.broadcast_to(piv, (8, 128))
            a1 = a2 = None
            for n, r in enumerate(range(0, D, 64)):
                p = piv if gate is None else gated(piv8, gate(n * gstep))[0:1]
                v = ld(r, 64) - p
                v1 = v[:32] + v[32:]
                v = v * v
                v2 = v[:32] + v[32:]
                a1 = v1 if a1 is None else a1 + v1
                a2 = v2 if a2 is None else a2 + v2
            s1, s2 = rowsum(a1) * (1.0 / D), rowsum(a2) * (1.0 / D)
            var = jnp.maximum(s2 - s1 * s1, 0.0)
            return piv + s1, lax.rsqrt(var + EPS)

        def ln_norm(ld, m, rstd, t):
            n = min(128, D - t * 128)
            blk = (ld(t * 128, n) - m) * rstd
            if n < 128:
                blk = jnp.concatenate([blk, jnp.zeros((128 - n, 128), f32)], axis=0)
            return blk.T

        def modulate(v, k, sl):
            return (v * mod_s[2 * k, 0:1, sl] + mod_s[2 * k + 1, 0:1, sl]).astype(bf16)

        def ln_apply(ld, m, rstd, k, dst, c):
            outs = []
            for t in range(5):
                sl = slice(t * 128, (t + 1) * 128)
                hb = modulate(ln_norm(ld, m, rstd, t), k, sl)
                outs.append(st16(dst, c * 128, (c + 1) * 128, sl, hb)[56:])
            return outs

        ALLC = tuple(range(TM // 128))
        ln2_stats = {}

        def xld(j, c):
            return lambda r, n: xt_s[j, r:r + n, c * 128:(c + 1) * 128].astype(f32)

        def ln1(j, dst, c, gate):
            ld = xld(j, c)
            return ln_apply(ld, *ln_stats(ld, gate), 0, dst, c)

        def ln2(c, gate):
            m, rstd = ln2_stats[c]
            m = gated(jnp.broadcast_to(m, (8, 128)), gate(0))[0:1]
            return ln_apply(lambda r, n: x1n_s[r:r + n, c * 128:(c + 1) * 128], m, rstd, 1, h2n_s, c)

        def padrow(r):
            return jnp.concatenate([r, jnp.zeros((r.shape[0], DP - D), f32)], axis=1)

        def colbcast(row):
            return jnp.broadcast_to(row, (128, DP)).T[:D]

        def matvec(ld, gate):
            acc = None
            for n, r in enumerate(range(0, D, 64)):
                sv = scol_s[r:r + 64, :]
                if gate is not None:
                    sv = gated(sv, gate(n * gstep))
                v = ld(r, 64).astype(f32) * sv
                v = v[:32] + v[32:]
                acc = v if acc is None else acc + v
            return rowsum(acc)

        def kvref(j):
            return stg_s if isinstance(j, int) and j == 1 else kv_s.at[j]

        def qkv_store(j, qkv, t0, t1):
            for t in range(t0, t1):
                v = qkv[:, (t - t0) * 128:(t - t0 + 1) * 128]
                if t < 4 or t == 13:
                    v = v * (DH ** -0.5 * LOG2E)
                kvref(j)[t, HALO:HALO + TM, :] = v
                if t >= 4:
                    kvref(j + 1)[t, :HALO, :] = v[TM - HALO:]

        def qkv_dots(j, src, parts, n=None, kt=-1):
            k0, k1 = (0, 5) if n is None else (KCH[n][0], KCH[n][0] + 1)
            st = {}

            def mk(t0, t1):
                def dot(tief):
                    if 'h' not in st:
                        st['h'] = ld16(src, 0, TM, k0 * 128, k1 * 128)
                    st['h'] = tief(st['h'])
                    if (t0, t1) == (4, 8):
                        res = jnp.dot(st['h'], ld16(wqn_s, k0 * 128, k1 * 128), preferred_element_type=f32)
                    else:
                        wq = ld16(wqt_s, t0 * 128, t1 * 128, k0 * 128, k1 * 128)
                        res = lax.dot_general(st['h'], wq, NT, preferred_element_type=f32)
                    acc = res if not n else res + part_s[j, :, t0 * 128:t1 * 128]
                    if n is not None and n < NK - 1:
                        part_s[j, :, t0 * 128:t1 * 128] = acc
                    else:
                        qkv_store(j, acc, t0, t1)
                    if t0 == kt:
                        ktl = lax.dot_general(ld16(wqt_s, 13 * 128, 13 * 128 + 64), st['h'], NT,
                                              preferred_element_type=f32)
                        qkv_store(j, jnp.concatenate([ktl, jnp.zeros((64, TM), f32)], axis=0).T, 13, 14)
                    return res
                return dot
            return [mk(*p) for p in parts]

        def attn_chunk(first, src, r, gate, jnext):
            r0 = r * RC
            q = [gated(src[t, HALO + r0:HALO + r0 + RC, :], gate) for t in Q_TILES]
            even = (lax.broadcasted_iota(jnp.int32, (RC, 128), 1) & 1) == 0
            ls = []
            for w in range(W):
                a = HALO + r0 - DIL * w
                p = q[0] * src[K_TILES[0], a:a + RC, :]
                for t in range(1, 5):
                    p = p + q[t] * src[K_TILES[t], a:a + RC, :]
                p = p + pltpu.roll(p, 64, 1)
                p = p + jnp.where(even, pltpu.roll(p, 127, 1), pltpu.roll(p, 1, 1))
                if first and r0 < DIL * w:
                    pos = r0 + lax.broadcasted_iota(jnp.int32, (RC, 128), 0)
                    p = jnp.where(pos >= DIL * w, p, -1e9 * LOG2E)
                ls.append(p)
            m = ls[0]
            for w in range(1, W):
                m = jnp.maximum(m, ls[w])
            es = [jnp.exp2(l - m) for l in ls]
            inv = 1.0 / _tree_sum(es)
            outs = []
            for t in range(5):
                acc = None
                for w in range(W):
                    a = HALO + r0 - DIL * w
                    term = es[w] * src[V_TILES[t], a:a + RC, :]
                    acc = term if acc is None else acc + term
                ob = (acc * inv).astype(bf16)
                outs.append(st16(o_s, r0, r0 + RC, slice(t * 128, (t + 1) * 128), ob))
            if jnext is None:
                return outs
            z = mkgate(outs)
            r1 = r0 + RC if r0 + RC < TM else TM + HALO
            for t in range(14):
                lo = max(r0, HALO) if t < 4 else r0
                if lo < r1:
                    v = gated(kv_s[jnext, t, lo:r1, :], z)
                    stg_s[t, lo:r1, :] = v
                    outs.append(v[:8])
            return outs

        def wo_dot(j):
            def dot(tief):
                attn_t = lax.dot_general(tief(ld16(wot_s, 0, D)), ld16(o_s, 0, TM), NT, preferred_element_type=f32)
                ga = jnp.concatenate([gcol_s[0]] * len(ALLC), axis=1)
                x1 = xt_s[j].astype(f32) + ga * attn_t
                x1n_s[...] = x1
                for c in ALLC:
                    ln2_stats[c] = ln_stats(lambda r, m: x1[r:r + m, c * 128:(c + 1) * 128], None)
                return attn_t
            return dot

        def wq_prep(k):
            r0, r1 = k * 128, min((k + 1) * 128, D)
            for s in range(14):
                if s < 13:
                    blk = wraw_s[r0:r1, s * 128:(s + 1) * 128]
                else:
                    blk = jnp.concatenate([wraw_s[r0:r1, s * 128:], jnp.zeros((r1 - r0, 64), bf16)], axis=1)
                if r1 - r0 < 128:
                    blk = jnp.concatenate([blk, jnp.zeros((128 - (r1 - r0), 128), bf16)], axis=0)
                tmp_s[k, s * 64:(s + 1) * 64, :] = pltpu.bitcast(blk.T, u32)
            for t in range(14):
                rows = [tmp_s[k, pl.ds(_pair_src(t, g), H, stride=DH // 2), :] for g in range(2) if _pair_src(t, g) >= 0]
                rows = jnp.concatenate(rows, axis=0)
                wqt_s[t * 64:t * 64 + rows.shape[0], k * 128:(k + 1) * 128] = rows

        def wq_untr(k, gate):
            outs = []
            for t in range(4, 8):
                rows = gated(wqt_s[t * 64:(t + 1) * 64, k * 128:(k + 1) * 128], gate)
                bits = st16(wqn_s, k * 128, (k + 1) * 128, slice((t - 4) * 128, (t - 3) * 128), pltpu.bitcast(rows, bf16).T)
                outs.append(bits[56:])
            return outs

        def wo_cvt(gate):
            outs = []
            for cc in range(5):
                if cc < 4:
                    v = wo_s[:, cc * 128:(cc + 1) * 128]
                else:
                    v = jnp.concatenate([wo_s[:, cc * 128:], jnp.zeros((D, 64), bf16)], axis=1)
                v = gated(pltpu.bitcast(v, u32), gate(cc * 48))
                tmp_s[cc, :D // 2, :] = v
                outs.append(v[D // 2 - 8:])
            return outs

        def wo_perm(t, gate):
            rows = []
            for g in range(2):
                s0 = _pair_src(V_TILES[t], g) - D
                if s0 >= 0:
                    rows.append(jnp.concatenate(
                        [gated(tmp_s[cc, pl.ds(s0, H, stride=DH // 2), :], gate) for cc in range(5)], axis=1))
                else:
                    rows.append(jnp.zeros((H, DP), u32))
            blk = pltpu.bitcast(jnp.concatenate(rows, axis=0), bf16).T[:D]
            bits = st16(wot_s, 0, D, slice(t * 128, (t + 1) * 128), blk)
            return [bits[k:k + 8] for k in (56, 120, 184, 248, 280)]

        def attn_task(first, src, r, jnext):
            return lambda gt: attn_chunk(first, src, r, gt(0), jnext)

        def ln1_task(j, dst, c):
            return lambda gt: ln1(j, dst, c, gt)

        def untr_task(k):
            return lambda gt: wq_untr(k, gt(0))

        def ident(h):
            return h

        start(g_first)
        start(g_k[0])
        start(g_second)
        for g in g_k[1:]:
            start(g)
        for jj in range(NLOOP):
            start(g_loop(jj))

        kv_s[0, 4:, :HALO, :] = jnp.zeros((10, HALO, 128), f32)
        zero_s[...] = jnp.zeros((8, 128), u32)
        wait(g_first)
        cvec = c_s[...].astype(f32)
        sc = (cvec * jax.nn.sigmoid(cvec)).astype(bf16)
        scol_s[...] = colbcast(padrow(sc.astype(f32)))

        st01, n01, mt = {}, {}, {}

        def norm_rows(j):
            for cc in ALLC:
                st01[j, cc] = ln_stats(xld(j, cc), None)
                n01[j, cc] = ln_norm(xld(j, cc), *st01[j, cc], KCH[0][0])

        def kprep(n, gate):
            k, mts = KCH[n]
            for t in mts:
                mt[t] = matvec(lambda r, m: wmod_s[r:r + m, t * 128:(t + 1) * 128], gate)
            sl = slice(k * 128, (k + 1) * 128)
            if k < 4:
                shift = mt[k]
                scale = 1.0 + jnp.concatenate([mt[4 + k][:, 64:], mt[5 + k][:, :64]], axis=1)
            else:
                z = jnp.zeros((1, 64), f32)
                shift = jnp.concatenate([mt[4][:, :64], z], axis=1)
                scale = jnp.concatenate([1.0 + mt[8][:, 64:], z], axis=1)
            mod_s[0, :, sl] = jnp.broadcast_to(scale, (8, 128))
            mod_s[1, :, sl] = jnp.broadcast_to(shift, (8, 128))
            wq_prep(k)

        def kh(n, j, dst):
            k = KCH[n][0]
            sl = slice(k * 128, (k + 1) * 128)
            for cc in ALLC:
                v = n01[j, cc] if n == 0 else ln_norm(xld(j, cc), *st01[j, cc], k)
                st16(dst, cc * 128, (cc + 1) * 128, sl, modulate(v, 0, sl))

        early, late = ((0, 4),), ((4, 8), (8, 12))
        norm_rows(0)
        for n in range(NK):
            wait(g_k[n])
            gate = None
            if n > 0:
                gate = gates([d(ident) for d in qkv_dots(1, hb_s, late, n - 1)][0], 0)
            kprep(n, gate)
            kh(n, 0, ha_s)
            if n == 0:
                wq_untr(KCH[0][0], None)
                wait(g_second)
                start(g_fin)
                start(g_gu)
                start(g_dn)
                for d in qkv_dots(0, ha_s, ((4, 8), (0, 4), (8, 12)), n):
                    d(ident)
                norm_rows(1)
                kh(n, 1, hb_s)
                for d in qkv_dots(1, hb_s, early, n):
                    d(ident)
                continue
            kh(n, 1, hb_s)
            if n < NK - 1:
                dots = qkv_dots(0, ha_s, ((0, 12),), n) + qkv_dots(1, hb_s, early, n)
                run_slots(dots, [[(untr_task(KCH[n][0]), 0)]], 0)
        dots = (qkv_dots(0, ha_s, ((0, 12),), NK - 1) + qkv_dots(0, ha_s, ((12, 13),), kt=12)
                + qkv_dots(1, hb_s, ((12, 13),), kt=12) + qkv_dots(1, hb_s, ((0, 12),), NK - 1))
        run_slots(dots, [[(ln1_task(2, hc_s, 0), l1g[0]), (ln1_task(2, hc_s, 1), l1g[1]), (untr_task(KCH[NK - 1][0]), l1g[2])]], 2)

        def abody(jj, _):
            wait(g_loop(jj))

            def mod2_task(t):
                def task(gate):
                    v = matvec(lambda r, n: wm2_s[jj, r:r + n, t * 128:(t + 1) * 128], gate)
                    v = jnp.broadcast_to(v, (8, 128))
                    mraw_s[jj, :, t * 128:(t + 1) * 128] = v
                    return [v]
                return task
            tasks = dict(A=[ln1_task(3 + jj, hc_s, 0)], B=[ln1_task(3 + jj, hc_s, 1)],
                         m=[mod2_task(t) for t in range(MW // 128)])
            run_slots(qkv_dots(2 + jj, hc_s, QS, kt=kt_at[0]), parse_plan(lplan, tasks), lag[0])
            return 0
        lax.fori_loop(0, NLOOP, abody, 0)

        wait(g_fin)

        def mod_fin(gate):
            z = gate(0)
            mod = jnp.concatenate([gated(mraw_s[jj, :, t * 128:(t + 1) * 128], z)
                                   for jj in range(NLOOP) for t in range(MW // 128)], axis=1)
            mod_s[2] = padrow(0.5 + 0.5 * mod[:, 2 * D:3 * D])
            mod_s[3] = padrow(0.5 * mod[:, D:2 * D])
            ga = colbcast(padrow(mod[0:1, :D]))
            gb = colbcast(padrow(2.0 * mod[0:1, 3 * D:]))
            gcol_s[0] = ga
            gcol_s[1] = gb
            return [g[k:k + 8] for g in (ga, gb) for k in (120, 248, 376, 504, 568)]

        d7 = qkv_dots(7, ha_s, QS, kt=kt_at[3])
        dots = (qkv_dots(5, hc_s, QS, kt=kt_at[1]) + qkv_dots(6, hb_s, QS, kt=kt_at[2])
                + d7[:wpos] + [wo_dot(0)] + d7[wpos:])
        tasks = dict(A=[ln1_task(6, hb_s, 0)], B=[ln1_task(6, hb_s, 1)], C=[ln1_task(7, ha_s, 0)],
                     D=[ln1_task(7, ha_s, 1)], M=[mod_fin], V=[wo_cvt],
                     X=[lambda gt: ln2(0, gt)], Y=[lambda gt: ln2(1, gt)],
                     a=[attn_task(True, kv_s.at[0], r, None) for r in range(TM // RC)],
                     p=[(lambda gt, t=t: wo_perm(t, gt(0))) for t in range(5)])
        run_slots(dots, parse_plan(fplan, tasks), lag[1])
        wait(g_gu)

        def glu(g, u):
            return ((g * u) * (1.0 + jnp.tanh(g))).astype(bf16)

        def act_cols(rows, c0):
            h = pltpu.bitcast(h2n_s[rows, :D], bf16)
            last = glu(jnp.dot(h, w1_s[:, F - LC:], preferred_element_type=f32),
                       jnp.dot(h, w3_s[:, F - LC:], preferred_element_type=f32))
            return lambda: jnp.concatenate([pltpu.bitcast(act_s[rows, c0:], bf16), last], axis=1)

        def bbody(i, _):
            j2 = jnp.minimum(i + 2, NB - 1)
            st = {'h': ld16(h2n_s, 0, TM, 0, D)}

            def keep_x1(gate):
                outs = []
                for n, r in enumerate(range(0, D, 64)):
                    for c in ALLC:
                        v = gated(x1n_s[r:r + 64, c * 128:(c + 1) * 128], gate(n * gstep))
                        x1_s[r:r + 64, c * 128:(c + 1) * 128] = v
                        outs.append(v[56:])
                return outs

            def gdot(sl):
                def dot(tief):
                    st['h'] = tief(st['h'])
                    st['g'] = jnp.dot(st['h'], w1_s[:, sl], preferred_element_type=f32)
                    return st['g']
                return dot

            def udot(sl):
                def dot(tief):
                    st['h'] = tief(st['h'])
                    u = jnp.dot(st['h'], w3_s[:, sl], preferred_element_type=f32)
                    st16(act_s, 0, TM, sl, glu(st['g'], u))
                    return u
                return dot
            dots = []
            for c0 in range(0, F - LC, FC):
                sl = slice(c0, min(c0 + FC, F - LC))
                dots += [gdot(sl), udot(sl)]
            plan = [[(attn_task(False, stg_s, r, j2), 0)] for r in range(TM // RC)]
            plan[xpos[0]].append((keep_x1, xpos[1]))
            run_slots(dots, plan, lag[2])

            @pl.when(i == 0)
            def _():
                wait(g_dn)

            @pl.when(i < NB - 1)
            def _():
                KS = ks * 128
                tail = act_cols(slice(0, TM // 2), 2 * KS)
                wo_dot(i + 1)(ident)
                w = w2t_s[...]
                y0 = lax.dot_general(w[:, :KS], ld16(act_s, 0, TM, 0, KS), NT, preferred_element_type=f32)
                outs = ln2(0, gates(y0, 0)) + ln2(1, gates(y0, 1))
                y1 = lax.dot_general(w[:, KS:2 * KS], ld16(act_s, 0, TM, KS, 2 * KS), NT, preferred_element_type=f32)
                y2 = lax.dot_general(tie(w[:, 2 * KS:], mkgate(outs)), tail(), NT, preferred_element_type=f32)
                gb = jnp.concatenate([gcol_s[1]] * len(ALLC), axis=1)
                out_s[i] = (x1_s[...] + gb * (y0 + y1 + y2)).astype(bf16)
                cp(out_s.at[i], o_hbm.at[:, pl.ds(i * TM, TM)], osem).start()
            return 0
        lax.fori_loop(0, NB, bbody, 0)

        def qbody(c, _):
            cols = pl.ds(pl.multiple_of(c * 128, 128), 128)
            ocols = pl.ds(pl.multiple_of((NB - 1) * TM + c * 128, 128), 128)
            a = act_cols(pl.ds(pl.multiple_of(c * 64, 64), 64), 0)()
            y = lax.dot_general(w2t_s[...], a, NT, preferred_element_type=f32)
            for r0, r1 in zip(qsp[:-1], qsp[1:]):
                out_s[NB - 1, r0:r1, cols] = (x1_s[r0:r1, cols] + gcol_s[1, r0:r1, :] * y[r0:r1]).astype(bf16)
                cp(out_s.at[NB - 1, r0:r1, cols], o_hbm.at[r0:r1, ocols], osem).start()
            return 0
        lax.fori_loop(0, TM // 128, qbody, 0)
        cp(o_hbm, o_hbm, osem).wait()

    def fn(A_x, A_wqkv, A_wo, B_x, B_w1, B_w3, B_w2, c, w_mod):
        hbm = pl.BlockSpec(memory_space=pltpu.HBM)
        V = pltpu.VMEM
        rows16 = V((TM // 2, DP), u32)
        out_t = pl.pallas_call(
            kern,
            in_specs=[hbm] * 8,
            out_specs=hbm,
            out_shape=jax.ShapeDtypeStruct((D, S), bf16),
            scratch_shapes=[
                V((NB, D, TM), bf16), V((D, 3 * D), bf16), V((5, 14 * 64, 128), u32), V((14 * 64, DP), u32), V((DP // 2, 512), u32),
                V((D, D), bf16), V((D // 2, DP), u32), V((1, D), bf16), V((D, 2 * D), bf16),
                V((NLOOP, D, MW), bf16), V((NLOOP, 8, MW), f32),
                V((D, F), bf16), V((D, F), bf16), V((D, F), bf16),
                V((4, 8, DP), f32), V((2, D, 128), f32), V((D, 128), f32), V((2, TM, 12 * 128), f32),
                V((14, TM + HALO, 128), f32), V((NB + 1, 14, TM + HALO + pk, 128), f32),
                rows16, rows16, rows16, rows16, V((D, TM), f32), V((D, TM), f32), rows16,
                V((8, 128), u32), V((TM // 2, F - LC), u32), V((NB, D, TM), bf16),
                pltpu.SemaphoreType.DMA((NK + 2 + NLOOP,)),
            ],
            compiler_params=pltpu.CompilerParams(vmem_limit_bytes=110 * 1024 * 1024, disable_bounds_checks=True),
        )(A_x[0].T, A_wqkv, A_wo, B_w1, B_w3, B_w2.T, c, w_mod)
        return out_t.T[None]
    return fn


_impl = make()


@jax.jit
def pallas_adaLN_cond__sliding_local_dilated__glu_gated_swiglu__prompt_kernel(
    A_x: jax.Array,
    A_wqkv: jax.Array,
    A_wo: jax.Array,
    B_x: jax.Array,
    B_w1: jax.Array,
    B_w3: jax.Array,
    B_w2: jax.Array,
    c: jax.Array,
    w_mod: jax.Array,
):
    return _impl(A_x, A_wqkv, A_wo, B_x, B_w1, B_w3, B_w2, c, w_mod)
```
